```python
import jax
import jax.numpy as jnp

def _softmax(x, axis=-1):
    return jax.nn.softmax(x, axis=axis)
def _gelu(x):
    return jax.nn.gelu(x, approximate=True)
def _silu(x):
    return jax.nn.silu(x)
def _sigmoid(x):
    return jax.nn.sigmoid(x)
def _layernorm(x, axis=-1, eps=1e-5):
    m = jnp.mean(x, axis=axis, keepdims=True)
    v = jnp.var(x, axis=axis, keepdims=True)
    return (x - m) / jnp.sqrt(v + eps)
def _scatter_add(tgt, idx, src, axis=0):
    return tgt.at[idx].add(src)
def _segment_sum(src, seg, n):
    return jax.ops.segment_sum(src, seg, n)
class _Rng:
    def __init__(self, key):
        self._k = key
    def _next(self):
        self._k, sub = jax.random.split(self._k)
        return sub
    def normal(self, shape):
        return jax.random.normal(self._next(), shape, dtype=jnp.bfloat16)
    def randint(self, lo, hi, shape):
        return jax.random.randint(self._next(), shape, lo, hi, dtype=jnp.int32)
    def uniform(self, shape, lo=0.0, hi=1.0):
        return jax.random.uniform(self._next(), shape, jnp.bfloat16, lo, hi)
    def permutation(self, n):
        return jax.random.permutation(self._next(), n)


kernel_name = 'interleave_layers__compressed_kv_cla__moe_arch_mod__decode'

def setup_inputs():
    _rng = _Rng(jax.random.key(int.from_bytes(__import__("os").urandom(4), "little")))
    _w = (lambda a: (lambda t: t.astype(jnp.bfloat16) if jnp.issubdtype(t.dtype, jnp.floating) else t)(jnp.asarray(a)))
    def _A_setup():
        B, H, Sq, Sk, D, M = 1, 32, 1, 4096, 128, 640
        Dc = 4 * D
        return {
            "x": _w((lambda *s: _rng.normal(s) * 0.05)(B, Sq, M)),
            "c_kv": _w((lambda *s: _rng.normal(s) * 0.05)(B, Sk, Dc)),
            "w_q": _w((lambda *s: _rng.normal(s) * 0.05)(M, H, D) * (M ** -0.5)),
            "w_uk": _w((lambda *s: _rng.normal(s) * 0.05)(Dc, H, D) * (Dc ** -0.5)),
            "w_uv": _w((lambda *s: _rng.normal(s) * 0.05)(Dc, H, D) * (Dc ** -0.5)),
            "w_o": _w((lambda *s: _rng.normal(s) * 0.05)(H, D, M) * ((H * D) ** -0.5)),
        }
    _A_in = _A_setup()

    def _B_setup():
        B, S, D, F, C = 1, 1, 640, 1728, 1
        return {
            "x": _w((lambda *s: _rng.normal(s) * 0.05)(B, S, D)),
            "w_r": _w((lambda *s: _rng.normal(s) * 0.05)(D)),
            "w_gate": _w((lambda *s: _rng.normal(s) * 0.05)(D, F)),
            "w_up": _w((lambda *s: _rng.normal(s) * 0.05)(D, F)),
            "w_down": _w((lambda *s: _rng.normal(s) * 0.05)(F, D)),
        }
    _B_in = _B_setup()

    return {
        "A_x": _A_in["x"],
        "A_c_kv": _A_in["c_kv"],
        "A_w_q": _A_in["w_q"],
        "A_w_uk": _A_in["w_uk"],
        "A_w_uv": _A_in["w_uv"],
        "A_w_o": _A_in["w_o"],
        "B_x": _B_in["x"],
        "B_w_r": _B_in["w_r"],
        "B_w_gate": _B_in["w_gate"],
        "B_w_up": _B_in["w_up"],
        "B_w_down": _B_in["w_down"],
    }

def reference(A_x, A_c_kv, A_w_q, A_w_uk, A_w_uv, A_w_o, B_x, B_w_r, B_w_gate, B_w_up, B_w_down):
    def _A_ref(x, c_kv, w_q, w_uk, w_uv, w_o):
        B, Sq, M = x.shape[0], x.shape[1], x.shape[2]
        Sk = c_kv.shape[1]
        H, D = w_q.shape[1], w_q.shape[2]
        q = jnp.einsum("bqm,mhd->bhqd", x, w_q)
        k = jnp.einsum("bkc,chd->bhkd", c_kv, w_uk)
        v = jnp.einsum("bkc,chd->bhkd", c_kv, w_uv)
        scores = jnp.einsum("bhqd,bhkd->bhqk", q, k) * (D ** -0.5)
        off = Sk - Sq
        qi = jnp.arange(Sq)[:, None]
        kj = jnp.arange(Sk)[None, :]
        cmask = kj <= (qi + off)
        scores = jnp.where(cmask[None, None], scores, -1e9)
        p = _softmax(scores, axis=-1)
        ctx = jnp.einsum("bhqk,bhkd->bhqd", p, v)
        return jnp.einsum("bhqd,hdm->bqm", ctx, w_o)

    def _B_ref(x, w_r, w_gate, w_up, w_down):
        B, S, D = x.shape
        C = 1
        r = x @ w_r
        idx = jnp.argsort(-r, axis=-1)[:, :C]
        idx_e = jnp.repeat(idx.reshape(B, C, 1), D, axis=2)
        x_sel = jnp.take_along_axis(x, idx_e, axis=1)
        g = _silu(x_sel @ w_gate)
        u = x_sel @ w_up
        y = (g * u) @ w_down
        r_sel = _sigmoid(jnp.take_along_axis(r, idx, axis=1))
        y = y * r_sel.reshape(B, C, 1)
        b_off = (jnp.arange(B) * S).reshape(B, 1)
        flat_idx = (idx + b_off).reshape(B * C)
        zero = (x * 0.0).reshape(B * S, D)
        upd = _scatter_add(zero, flat_idx, y.reshape(B * C, D), axis=0)
        return x + upd.reshape(B, S, D)

    x = A_x
    x = x + _A_ref(_layernorm(x, axis=-1), A_c_kv, A_w_q, A_w_uk, A_w_uv, A_w_o)
    x = x + _B_ref(_layernorm(x, axis=-1), B_w_r, B_w_gate, B_w_up, B_w_down)
    x = x + _A_ref(_layernorm(x, axis=-1), A_c_kv, A_w_q, A_w_uk, A_w_uv, A_w_o)
    x = x + _B_ref(_layernorm(x, axis=-1), B_w_r, B_w_gate, B_w_up, B_w_down)
    return x
```

```python
import functools
import math
import jax
import jax.numpy as jnp
from jax import lax
import jax.experimental.pallas as pl
import jax.experimental.pallas.tpu as pltpu

F32, BF16, I32 = jnp.float32, jnp.bfloat16, jnp.int32
M, H, D, SK, DC, F = 640, 32, 128, 4096, 512, 1728
NM = M // 128
NC = DC // 128
NK = SK // 128
NF = 14
WO_SPLIT = (0, 24, 32)
WD_SPLIT = (0, 2, 4, 5)
NWO = len(WO_SPLIT) - 1
NWD = len(WD_SPLIT) - 1
NN = (((1,), (0,)), ((), ()))
NT = (((1,), (1,)), ((), ()))


def _iota(shape, dim):
    return lax.broadcasted_iota(I32, shape, dim)


def _dot(a, b):
    return lax.dot_general(a, b, NN, preferred_element_type=F32)


def _dot_t(a, b):
    return lax.dot_general(a, b, NT, preferred_element_type=F32)


def _tile(ref, i):
    return pltpu.bitcast(ref[i], BF16)


def _words(v):
    return pltpu.bitcast(v.astype(BF16), I32)


def _kernel(x_hbm, wr_hbm, c_hbm, wq_hbm, wuk_hbm, wuv_hbm, wo_hbm, wg_hbm, wu_hbm, wd_hbm,
            o_ref,
            x_v, wr_v, c_v, wq_v, wuk_v, wuv_v, wo_v, wg_v, wu_v, wd_v,
            wq_t, wuk_t, wuv_t, c_t, gu_t, s_scr, z_scr, q_scr, ctx_scr, csq_scr, csgu_scr, sems):
    pairs = [(x_hbm, x_v), (wr_hbm, wr_v), (wq_hbm, wq_v), (wuk_hbm, wuk_v), (c_hbm, c_v),
             (wuv_hbm, wuv_v), (wg_hbm, wg_v), (wu_hbm, wu_v)]
    for h0, h1 in zip(WO_SPLIT[:-1], WO_SPLIT[1:]):
        rows = pl.ds(D * h0, D * (h1 - h0))
        pairs.append((wo_hbm.at[rows, :], wo_v.at[rows, :]))
    for j0, j1 in zip(WD_SPLIT[:-1], WD_SPLIT[1:]):
        cols = pl.ds(128 * j0, 128 * (j1 - j0))
        pairs.append((wd_hbm.at[:, cols], wd_v.at[:, cols]))
    cps = [pltpu.make_async_copy(s, d, sems.at[i]) for i, (s, d) in enumerate(pairs)]
    for cp in cps:
        cp.start()
    X, WR, WQ, WUK, C, WUV, WG, WU, WO = range(9)
    WD = WO + NWO

    sub = _iota((8, 128), 0)
    zero8 = jnp.zeros((8, 128), F32)
    eye = (_iota((128, 128), 0) == _iota((128, 128), 1)).astype(BF16)

    def row(r, v):
        return jnp.where(sub == r, v, 0.0)

    def head_pair(view, j):
        a = view[pl.ds(j, 64, stride=32), :]
        b = view[pl.ds(16 + j, 64, stride=32), :]
        return (a & 0xFFFF) | (b << 16), lax.shift_right_logical(a, 16) | (b & -65536)

    def split_heads(src_v, nblk, dst):
        w32 = src_v.bitcast(I32)

        def body(blk, carry):
            view = w32.at[pl.ds(pl.multiple_of(blk * 2048, 2048), 2048), :]
            for j in range(H // 2):
                lo, hi = head_pair(view, j)
                dst[(2 * j) * nblk + blk] = lo
                dst[(2 * j + 1) * nblk + blk] = hi
            return carry

        lax.fori_loop(0, nblk, body, 0)

    def transpose_gu(src_v, which):
        lhs = jnp.concatenate([eye, jnp.ones((16, 128), BF16)], axis=0)

        def do(tile, base, j):
            o = _dot_t(lhs, tile)
            gu_t[base + j] = _words(o[0:128])
            return o[128:136]

        def body(g, carry):
            css = []
            for i in range(4):
                ft = g * 4 + i
                r0 = pl.multiple_of(ft * 128, 128)
                cs = None
                for j in range(NM):
                    o = do(src_v[pl.ds(r0, 128), 128 * j:128 * (j + 1)], (which * NF + ft) * NM, j)
                    cs = o if cs is None else cs + o
                csgu_scr[which * NF + ft] = cs
            return carry

        lax.fori_loop(0, 3, body, 0)
        for ft in (NF - 2, NF - 1):
            cs = None
            for j in range(NM):
                t = src_v[128 * ft:min(128 * (ft + 1), F), 128 * j:128 * (j + 1)]
                if ft == NF - 1:
                    t = jnp.concatenate([t, jnp.zeros((128 * NF - F, 128), BF16)], axis=0)
                o = do(t, (which * NF + ft) * NM, j)
                cs = o if cs is None else cs + o
            csgu_scr[which * NF + ft] = cs

    def stats(xs):
        tot = xs[0]
        for v in xs[1:]:
            tot = tot + v
        mu = jnp.sum(tot, axis=-1, keepdims=True) * (1.0 / M)
        sq = None
        for v in xs:
            d = v - mu
            sq = d * d if sq is None else sq + d * d
        var = jnp.sum(sq, axis=-1, keepdims=True) * (1.0 / M)
        return mu, lax.rsqrt(var + 1e-5)

    ones_rows = [row(r, 1.0) for r in range(8)]

    def q_part(j, xj, acc, first):
        lhs = []
        for r in range(8):
            l = row(r, xj)
            if first:
                l = jnp.concatenate([l, ones_rows[r]], axis=0)
            lhs.append(l)
        for h in range(H):
            o = _dot(lhs[h % 8], _tile(wq_t, h * NM + j))
            acc[h // 8] = o if acc[h // 8] is None else acc[h // 8] + o

    QSCALE = D ** -0.5 * math.log2(math.e)

    def qabs(qs, rstd):
        scale = rstd * QSCALE
        zs = []
        for b in range(NC):
            z = [zero8] * 4
            for h in range(H):
                o = _dot(qs[h // 8], _tile(wuk_t, h * NC + b))
                z[h // 8] = jnp.where(sub == h % 8, o, z[h // 8])
            zs.append(jnp.concatenate([v * scale for v in z], axis=0).astype(BF16))
        return zs

    def qabs_first(rstd):
        w32 = wuk_v.bitcast(I32)
        scale = rstd * QSCALE

        def body(b, carry):
            view = w32.at[pl.ds(pl.multiple_of(b * 2048, 2048), 2048), :]
            z = [zero8] * 4
            for j in range(H // 2):
                a = j // 4
                qb = q_scr[16 * a:16 * a + 16, :]
                lhs = jnp.concatenate([eye, qb], axis=0)
                for e, w in enumerate(head_pair(view, j)):
                    h = 2 * j + e
                    o = _dot_t(lhs, pltpu.bitcast(w, BF16))
                    wuk_t[h * NC + b] = _words(o[0:128])
                    z[a] = jnp.where(sub == h % 8, o[128:136], z[a])
            z_scr[b] = jnp.concatenate([v * scale for v in z], axis=0)
            return carry

        lax.fori_loop(0, NC, body, 0)
        return [z_scr[b].astype(BF16) for b in range(NC)]

    def scores_first(zs):
        lhs = [jnp.concatenate([eye, zs[b]], axis=0) for b in range(NC)]
        U = 4

        def body(g, carry):
            for i in range(U):
                t = g * U + i
                r0 = pl.multiple_of(t * 128, 128)
                s = None
                for b in range(NC):
                    o = _dot_t(lhs[b], c_v[pl.ds(r0, 128), 128 * b:128 * (b + 1)])
                    c_t[b * NK + t] = _words(o[0:128])
                    s = o[128:160] if s is None else s + o[128:160]
                s_scr[t] = s
            return carry

        lax.fori_loop(0, NK // U, body, 0)

    HALF = NK // 2

    def scores(zs, t0):
        mx = None
        for g0 in range(t0, t0 + HALF, 4):
            acc = [None] * 4
            for b in range(NC):
                for i in range(4):
                    o = _dot(zs[b], _tile(c_t, b * NK + g0 + i))
                    acc[i] = o if acc[i] is None else acc[i] + o
            for i in range(4):
                s_scr[g0 + i] = acc[i]
                mx = acc[i] if mx is None else jnp.maximum(mx, acc[i])
        return jnp.max(mx, axis=-1, keepdims=True)

    def smax(t0):
        mx = None
        for t in range(t0, t0 + HALF):
            v = s_scr[t]
            mx = v if mx is None else jnp.maximum(mx, v)
        return jnp.max(mx, axis=-1, keepdims=True)

    def attention_tail(m_a, m_b, first):
        m = jnp.maximum(m_a, m_b)
        alpha = jnp.exp2(m_a - m)

        def cv(t, b):
            return c_v[128 * t:128 * (t + 1), 128 * b:128 * (b + 1)]

        acc = [None] * NC
        lsum = None
        for t in range(HALF):
            p = jnp.exp2(s_scr[t] - m_a)
            lsum = p if lsum is None else lsum + p
            pb = p.astype(BF16)
            for b in range(NC):
                o = _dot(pb, cv(t, b))
                acc[b] = o if acc[b] is None else acc[b] + o
        lsum = lsum * alpha
        acc = [v * alpha for v in acc]
        for t in range(HALF, HALF + 8):
            p = jnp.exp2(s_scr[t] - m)
            lsum = lsum + p
            pb = p.astype(BF16)
            for b in range(NC):
                acc[b] = acc[b] + _dot(pb, cv(t, b))
        pbs = {}
        for b in range(NC):
            for t in range(HALF + 8, NK):
                if b == 0:
                    p = jnp.exp2(s_scr[t] - m)
                    lsum = lsum + p
                    pbs[t] = p.astype(BF16)
                acc[b] = acc[b] + _dot(pbs[t], cv(t, b))
        linv = 1.0 / jnp.sum(lsum, axis=-1, keepdims=True)
        if first:
            cps[WUV].wait()
            split_heads(wuv_v, NC, wuv_t)
        ctx = [None] * 4
        for b in range(NC):
            for h in range(H):
                a, r = divmod(h, 8)
                o = _dot(row(r, acc[b][8 * a:8 * a + 8]), _tile(wuv_t, h * NC + b))
                ctx[a] = o if ctx[a] is None else ctx[a] + o
        for a in range(4):
            ctx_scr[8 * a:8 * a + 8, :] = ctx[a] * linv[8 * a:8 * a + 8]
        if first:
            cps[WG].wait()
            transpose_gu(wg_v, 0)
            cps[WU].wait()
            transpose_gu(wu_v, 1)

        def o_tile(h, j):
            l = jnp.broadcast_to(ctx_scr[h:h + 1, :], (8, 128))
            return _dot(l, wo_v[128 * h:128 * (h + 1), 128 * j:128 * (j + 1)])

        outs = [None] * NM
        if first:
            for i in range(NWO):
                cps[WO + i].wait()
                for h in range(WO_SPLIT[i], WO_SPLIT[i + 1]):
                    for j in range(NM):
                        t = o_tile(h, j)
                        outs[j] = t if outs[j] is None else outs[j] + t
        else:
            for j in range(NM):
                for h in range(H):
                    t = o_tile(h, j)
                    outs[j] = t if outs[j] is None else outs[j] + t
        return outs

    def ffn_act(xs, mu, rstd):
        acts = [None] * NF
        for f0 in range(0, NF, 2):
            fts = [f0, f0 + 1]
            acc = {}
            for j in range(NM):
                for ft in fts:
                    for which in range(2):
                        o = _dot(xs[j], _tile(gu_t, (which * NF + ft) * NM + j))
                        acc[ft, which] = o if j == 0 else acc[ft, which] + o
            for ft in fts:
                g = rstd * (acc[ft, 0] - mu * csgu_scr[ft])
                u = rstd * (acc[ft, 1] - mu * csgu_scr[NF + ft])
                acts[ft] = g * jax.nn.sigmoid(g) * u
        return acts

    def wd_tile(ft, j):
        t = wd_v[128 * ft:min(128 * (ft + 1), F), 128 * j:128 * (j + 1)]
        if ft == NF - 1:
            t = jnp.concatenate([t, jnp.zeros((128 * NF - F, 128), BF16)], axis=0)
        return t

    def ffn_residual(xs, mu, rstd, wr):
        xn = [((v - mu) * rstd).astype(BF16).astype(F32) for v in xs]
        rr = None
        for v, w in zip(xn, wr):
            rr = v * w if rr is None else rr + v * w
        sig = jax.nn.sigmoid(jnp.sum(rr, axis=-1, keepdims=True))
        base = [v + n for v, n in zip(xs, xn)]
        zero = [n * 0.0 for n in xn]
        return base, zero, sig

    cps[X].wait()
    cps[WR].wait()
    x_all = jnp.broadcast_to(x_v[...].astype(F32), (8, M))
    wr_all = jnp.broadcast_to(wr_v[...].reshape(1, M).astype(F32), (8, M))
    xs = [x_all[:, 128 * j:128 * (j + 1)] for j in range(NM)]
    wr = [wr_all[:, 128 * j:128 * (j + 1)] for j in range(NM)]
    mu, rstd = stats(xs)

    cps[WQ].wait()
    split_heads(wq_v, NM, wq_t)
    qacc = [None] * 4
    for j in range(NM):
        q_part(j, xs[j], qacc, True)
    for a in range(4):
        cs = qacc[a][8:16]
        csq_scr[8 * a:8 * a + 8, :] = cs
        q_scr[16 * a:16 * a + 16, :] = jnp.concatenate([qacc[a][0:8] - mu * cs, zero8], axis=0).astype(BF16)
    cps[WUK].wait()
    zs = qabs_first(rstd)
    cps[C].wait()
    scores_first(zs)
    outs = attention_tail(smax(0), smax(HALF), True)
    xs = [v + o for v, o in zip(xs, outs)]
    mu, rstd = stats(xs)
    acts = ffn_act(xs, mu, rstd)
    base, zero, sig = ffn_residual(xs, mu, rstd, wr)
    qacc = [None] * 4
    xs = []
    for j in range(NM):
        if j in WD_SPLIT:
            cps[WD + WD_SPLIT.index(j)].wait()
        y = None
        for ft in range(NF):
            o = _dot(acts[ft], wd_tile(ft, j))
            y = o if y is None else y + o
        xs.append(base[j] + (zero[j] + y * sig))
        q_part(j, xs[j], qacc, False)

    mu, rstd = stats(xs)
    qs = [qacc[a] - mu * csq_scr[8 * a:8 * a + 8, :] for a in range(4)]
    zs = qabs(qs, rstd)
    m_a = scores(zs, 0)
    m_b = scores(zs, HALF)
    outs = attention_tail(m_a, m_b, False)
    xs = [v + o for v, o in zip(xs, outs)]
    mu, rstd = stats(xs)
    acts = ffn_act(xs, mu, rstd)
    base, zero, sig = ffn_residual(xs, mu, rstd, wr)
    ys = [None] * NM
    for ft in range(NF):
        for j in range(NM):
            o = _dot(acts[ft], wd_tile(ft, j))
            ys[j] = o if ys[j] is None else ys[j] + o
    for j in range(NM):
        xo = base[j] + (zero[j] + ys[j] * sig)
        o_ref[:, 128 * j:128 * (j + 1)] = xo[0:1, :].astype(o_ref.dtype)


@jax.jit
def pallas_interleave_layers__compressed_kv_cla__moe_arch_mod__decode_kernel(
        A_x, A_c_kv, A_w_q, A_w_uk, A_w_uv, A_w_o, B_x, B_w_r, B_w_gate, B_w_up, B_w_down):
    del B_x
    any_spec = pl.BlockSpec(memory_space=pl.ANY)
    out = pl.pallas_call(
        _kernel,
        out_shape=jax.ShapeDtypeStruct((1, M), BF16),
        in_specs=[any_spec] * 10,
        out_specs=pl.BlockSpec(memory_space=pltpu.VMEM),
        scratch_shapes=[
            pltpu.VMEM((1, M), BF16), pltpu.VMEM((M,), BF16),
            pltpu.VMEM((SK, DC), BF16),
            pltpu.VMEM((M * H, D), BF16), pltpu.VMEM((DC * H, D), BF16), pltpu.VMEM((DC * H, D), BF16),
            pltpu.VMEM((H * D, M), BF16),
            pltpu.VMEM((F, M), BF16), pltpu.VMEM((F, M), BF16), pltpu.VMEM((F, M), BF16),
            pltpu.VMEM((H * NM, 64, 128), I32), pltpu.VMEM((H * NC, 64, 128), I32),
            pltpu.VMEM((H * NC, 64, 128), I32), pltpu.VMEM((NC * NK, 64, 128), I32),
            pltpu.VMEM((2 * NF * NM, 64, 128), I32),
            pltpu.VMEM((NK, H, 128), F32), pltpu.VMEM((NC, H, 128), F32), pltpu.VMEM((2 * H, D), BF16),
            pltpu.VMEM((H, D), F32), pltpu.VMEM((H, D), F32),
            pltpu.VMEM((2 * NF, 8, 128), F32),
            pltpu.SemaphoreType.DMA((8 + NWO + NWD,)),
        ],
        compiler_params=pltpu.CompilerParams(vmem_limit_bytes=100 * 2**20),
    )(A_x.reshape(1, M), B_w_r, A_c_kv.reshape(SK, DC), A_w_q.reshape(M * H, D),
      A_w_uk.reshape(DC * H, D), A_w_uv.reshape(DC * H, D), A_w_o.reshape(H * D, M),
      B_w_gate.T, B_w_up.T, B_w_down)
    return out.reshape(1, 1, M)
```

```python
import math
import jax
import jax.numpy as jnp
from jax import lax
import jax.experimental.pallas as pl
import jax.experimental.pallas.tpu as pltpu

F32, BF16, I32 = jnp.float32, jnp.bfloat16, jnp.int32
M, H, D, SK, DC, F = 640, 32, 128, 4096, 512, 1728
NM = M // 128
NC = DC // 128
NK = SK // 128
NF = 14
WO_SPLIT = (0, 12, 24, 32)
WD_SPLIT = (0, 2, 4, 5)
NWO = len(WO_SPLIT) - 1
NWD = len(WD_SPLIT) - 1
NN = (((1,), (0,)), ((), ()))
NT = (((1,), (1,)), ((), ()))

QV = tuple(range(12))
VV = tuple(range(20, 32))
OV = tuple(range(12))
GV = tuple(range(8, 14))
VM = (0, 1, 2, 3, 4, 5, 12, 13, 14, 15, 16, 17, 18, 19, 6, 7, 8, 9, 10, 11)
OM = (20, 21, 22, 23, 24, 25, 26, 27, 28, 12, 13, 14, 15, 16, 17, 18, 19, 29, 30, 31)
DV = ()
DG = 3
DLAG = 10
QG = 3
OG = 3
QLAG = 10
OLAG = 10
GLAG = 9
VLAG = 4
SLEAD = 2
VGATE = 0
QM = tuple(h for h in range(H) if h not in QV)
GM = tuple(f for f in range(NF) if f not in GV)
assert sorted(VM + VV) == list(range(H)) and sorted(OM + OV) == list(range(H))


def _iota(shape, dim):
    return lax.broadcasted_iota(I32, shape, dim)


def _dot(a, b):
    return lax.dot_general(a, b, NN, preferred_element_type=F32)


def _dot_t(a, b):
    return lax.dot_general(a, b, NT, preferred_element_type=F32)


def _tile(ref, i):
    return pltpu.bitcast(ref[i], BF16)


def _words(v):
    return pltpu.bitcast(v.astype(BF16), I32)


def _interleave(mx, vp):
    nm, nv = len(mx), len(vp)
    iv = 0
    for im, step in enumerate(mx):
        step()
        while iv < (im + 1) * nv // nm:
            vp[iv]()
            iv += 1
    while iv < nv:
        vp[iv]()
        iv += 1


def _rowsum(v):
    return jnp.broadcast_to(jnp.sum(v, axis=0, keepdims=True), v.shape)


def _columns(rowvec):
    return jnp.broadcast_to(rowvec[0:1, :], (128, 128)).T


def _kernel(x_hbm, wr_hbm, c_hbm, wq_hbm, wuk_hbm, wuv_hbm, wo_hbm, wg_hbm, wu_hbm, wd_hbm,
            o_ref,
            x_v, wr_v, c_v, wq_v, wuk_v, wuv_v, wo_v, wg_v, wu_v, wd_v,
            wq_t, wuk_t, wuk_f, wuv_t, wuv_f, wo_t, wo_f, c_t, gu_t, gu_f,
            s_scr, z_scr, q_scr, a_scr, ctx_scr, ctxv_scr, csq_scr, csgu_scr, sems):
    pairs = {"wq": (wq_hbm, wq_v), "x": (x_hbm, x_v), "wr": (wr_hbm, wr_v), "wuk": (wuk_hbm, wuk_v),
             "c": (c_hbm, c_v), "wuv": (wuv_hbm, wuv_v), "wg": (wg_hbm, wg_v), "wu": (wu_hbm, wu_v)}
    for i, (h0, h1) in enumerate(zip(WO_SPLIT[:-1], WO_SPLIT[1:])):
        rows = pl.ds(D * h0, D * (h1 - h0))
        pairs["wo", i] = (wo_hbm.at[rows, :], wo_v.at[rows, :])
    for i, (j0, j1) in enumerate(zip(WD_SPLIT[:-1], WD_SPLIT[1:])):
        cols = pl.ds(128 * j0, 128 * (j1 - j0))
        pairs["wd", i] = (wd_hbm.at[:, cols], wd_v.at[:, cols])
    order = ["wq", "x", "wr", "wuk", "c", "wuv", ("wo", 0), "wg", "wu"]
    order += [("wo", i) for i in range(1, NWO)] + [("wd", i) for i in range(NWD)]
    cps = {k: pltpu.make_async_copy(*pairs[k], sems.at[i]) for i, k in enumerate(order)}
    for k in order:
        cps[k].start()

    sub = _iota((8, 128), 0)
    lane = _iota((8, 128), 1)
    zero8 = jnp.zeros((8, 128), F32)
    eye = (_iota((128, 128), 0) == _iota((128, 128), 1)).astype(BF16)

    def row(r, v):
        return jnp.where(sub == r, v, 0.0)

    def bcast_row(ref, r, c0=0):
        return jnp.broadcast_to(ref[r:r + 1, c0:c0 + 128], (8, 128))

    def head_pair(view, j):
        a = view[pl.ds(j, 64, stride=32), :]
        b = view[pl.ds(16 + j, 64, stride=32), :]
        return (a & 0xFFFF) | (b << 16), lax.shift_right_logical(a, 16) | (b & -65536)

    def split_wq():
        w32 = wq_v.bitcast(I32)

        def body(blk, carry):
            view = w32.at[pl.ds(pl.multiple_of(blk * 2048, 2048), 2048), :]
            for j in range(H // 2):
                lo, hi = head_pair(view, j)
                wq_t[(2 * j) * NM + blk] = lo
                wq_t[(2 * j + 1) * NM + blk] = hi
            return carry

        lax.fori_loop(0, NM, body, 0)

    def split_wuv():
        w32 = wuv_v.bitcast(I32)

        def body(b, carry):
            view = w32.at[pl.ds(pl.multiple_of(b * 2048, 2048), 2048), :]
            for j in range(H // 2):
                pair = head_pair(view, j)
                for e in range(2):
                    h = 2 * j + e
                    if h in VM:
                        wuv_t[VM.index(h) * NC + b] = pair[e]
                    else:
                        t = _dot_t(eye, pltpu.bitcast(pair[e], BF16))
                        for i in range(16):
                            wuv_f[(VV.index(h) * 16 + i) * NC + b] = t[8 * i:8 * i + 8]
            return carry

        lax.fori_loop(0, NC, body, 0)

    def transpose_gu(src_v, which):
        lhs = jnp.concatenate([eye, jnp.ones((16, 128), BF16)], axis=0)
        NTV = 2 * len(GV)

        def do(tile, ft, j):
            o = _dot_t(lhs, tile)
            if ft in GM:
                gu_t[(which * len(GM) + GM.index(ft)) * NM + j] = _words(o[0:128])
            else:
                for g in range(16):
                    gu_f[(j * 16 + g) * NTV + 2 * GV.index(ft) + which] = o[8 * g:8 * g + 8]
            return o[128:136]

        def body(j, carry):
            cols = pl.ds(pl.multiple_of(j * 128, 128), 128)
            css = []
            for ft in range(NF):
                t = src_v[128 * ft:min(128 * (ft + 1), F), cols]
                if ft == NF - 1:
                    t = jnp.concatenate([t, jnp.zeros((128 * NF - F, 128), BF16)], axis=0)
                css.append(carry[ft] + do(t, ft, j))
            return tuple(css)

        css = lax.fori_loop(0, NM, body, (zero8,) * NF)
        for ft in range(NF):
            csgu_scr[which * NF + ft] = css[ft]

    def column_stream(groups, prep, mac, lag):
        cols = {}
        steps = []

        def start(i, dep):
            if i < len(groups):
                for key in groups[i]:
                    cols[key] = _columns(prep(key, dep))

        def make(i, g):
            def step():
                if i == 0 and g == 0:
                    start(0, None)
                    start(1, None)
                last = None
                for key in groups[i]:
                    last = mac(key, g, cols[key][8 * g:8 * g + 8])
                if g == lag:
                    start(i + 2, last)
            return step

        for i in range(len(groups)):
            for g in range(16):
                steps.append(make(i, g))
        return steps

    def stats(xs):
        tot = xs[0]
        for v in xs[1:]:
            tot = tot + v
        mu = jnp.sum(tot, axis=-1, keepdims=True) * (1.0 / M)
        sq = None
        for v in xs:
            d = v - mu
            sq = d * d if sq is None else sq + d * d
        var = jnp.sum(sq, axis=-1, keepdims=True) * (1.0 / M)
        return mu, lax.rsqrt(var + 1e-5)

    ones_rows = [row(r, 1.0) for r in range(8)]

    def q_part(j, xj, acc, first):
        lhs = []
        for r in range(8):
            l = row(r, xj)
            if first:
                l = jnp.concatenate([l, ones_rows[r]], axis=0)
            lhs.append(l)
        for h in range(H):
            o = _dot(lhs[h % 8], _tile(wq_t, h * NM + j))
            acc[h // 8] = o if acc[h // 8] is None else acc[h // 8] + o

    QSCALE = D ** -0.5 * math.log2(math.e)

    def qabs(qs, rstd):
        scale = rstd * QSCALE
        z = [[zero8] * 4 for _ in range(NC)]

        def mstep(b, h):
            def step():
                o = _dot(qs[h // 8], _tile(wuk_t, QM.index(h) * NC + b))
                z[b][h // 8] = jnp.where(sub == h % 8, o, z[b][h // 8])
            return step

        vqacc = {}
        groups = [QV[k:k + QG] for k in range(0, len(QV), QG)]

        def prep_q(h, dep):
            src = _rowsum(row(h % 8, qs[h // 8]))
            return src if dep is None else after(dep, src)

        def q_mac(h, g, m):
            for b in range(NC):
                p = m * wuk_f[(QV.index(h) * 16 + g) * NC + b]
                vqacc[h, b] = p if g == 0 else vqacc[h, b] + p
                if g == 15:
                    z[b][h // 8] = jnp.where(sub == h % 8, _rowsum(vqacc[h, b]), z[b][h // 8])
            return vqacc[h, NC - 1]

        _interleave([mstep(b, h) for b in range(NC) for h in QM],
                    column_stream(groups, prep_q, q_mac, QLAG))
        return [jnp.concatenate([v * scale for v in z[b]], axis=0).astype(BF16) for b in range(NC)]

    def qabs_first(rstd):
        w32 = wuk_v.bitcast(I32)
        scale = rstd * QSCALE

        def body(b, carry):
            view = w32.at[pl.ds(pl.multiple_of(b * 2048, 2048), 2048), :]
            z = [zero8] * 4
            for j in range(H // 2):
                a = j // 4
                qb = q_scr[16 * a:16 * a + 16, :]
                lhs = jnp.concatenate([eye, qb], axis=0)
                for e, w in enumerate(head_pair(view, j)):
                    h = 2 * j + e
                    o = _dot_t(lhs, pltpu.bitcast(w, BF16))
                    if h in QM:
                        wuk_t[QM.index(h) * NC + b] = _words(o[0:128])
                    else:
                        for g in range(16):
                            wuk_f[(QV.index(h) * 16 + g) * NC + b] = o[8 * g:8 * g + 8]
                    z[a] = jnp.where(sub == h % 8, o[128:136], z[a])
            z_scr[b] = jnp.concatenate([v * scale for v in z], axis=0)
            return carry

        lax.fori_loop(0, NC, body, 0)
        return [z_scr[b].astype(BF16) for b in range(NC)]

    def scores_first(zs):
        lhs = [jnp.concatenate([eye, zs[b]], axis=0) for b in range(NC)]
        U = 4

        def body(g, carry):
            for i in range(U):
                t = g * U + i
                r0 = pl.multiple_of(t * 128, 128)
                s = None
                for b in range(NC):
                    o = _dot_t(lhs[b], c_v[pl.ds(r0, 128), 128 * b:128 * (b + 1)])
                    c_t[b * NK + t] = _words(o[0:128])
                    s = o[128:160] if s is None else s + o[128:160]
                s_scr[t] = s
            return carry

        lax.fori_loop(0, NK // U, body, 0)

    HALF = NK // 2

    def scores(zs, t0):
        mx = None
        acc = {}

        def tile(t, b):
            o = _dot(zs[b], _tile(c_t, b * NK + t))
            acc[t] = o if b == 0 else acc[t] + o

        groups = [list(range(g0, g0 + 4)) for g0 in range(t0, t0 + HALF, 4)]
        if t0 == 0:
            for b in range(NC - 1):
                for grp in groups[:SLEAD]:
                    for t in grp:
                        tile(t, b)
            for grp in groups[:SLEAD]:
                for t in grp:
                    tile(t, NC - 1)
        for k, grp in enumerate(groups):
            if t0 != 0 or k >= SLEAD:
                for b in range(NC):
                    for t in grp:
                        tile(t, b)
            for t in grp:
                s_scr[t] = acc[t]
                mx = acc[t] if mx is None else jnp.maximum(mx, acc[t])
        return jnp.max(mx, axis=-1, keepdims=True)

    def smax(t0):
        mx = None
        for t in range(t0, t0 + HALF):
            v = s_scr[t]
            mx = v if mx is None else jnp.maximum(mx, v)
        return jnp.max(mx, axis=-1, keepdims=True)

    def softmax_pv(m_a, m_b):
        m = jnp.maximum(m_a, m_b)
        alpha = jnp.exp2(m_a - m)

        def cv(t, b):
            return c_v[128 * t:128 * (t + 1), 128 * b:128 * (b + 1)]

        acc = [None] * NC
        lsum = None
        for t in range(HALF):
            p = jnp.exp2(s_scr[t] - m_a)
            lsum = p if lsum is None else lsum + p
            pb = p.astype(BF16)
            for b in range(NC):
                o = _dot(pb, cv(t, b))
                acc[b] = o if acc[b] is None else acc[b] + o
        lsum = lsum * alpha
        acc = [v * alpha for v in acc]
        for t in range(HALF, HALF + 8):
            p = jnp.exp2(s_scr[t] - m)
            lsum = lsum + p
            pb = p.astype(BF16)
            for b in range(NC):
                acc[b] = acc[b] + _dot(pb, cv(t, b))
        pbs = {}
        for b in range(NC):
            for t in range(HALF + 8, NK):
                if b == 0:
                    p = jnp.exp2(s_scr[t] - m)
                    lsum = lsum + p
                    pbs[t] = p.astype(BF16)
                acc[b] = acc[b] + _dot(pbs[t], cv(t, b))
        linv = 1.0 / jnp.sum(lsum, axis=-1, keepdims=True)
        return acc, linv

    def context(acc, linv):
        for b in range(NC):
            a_scr[:, 128 * b:128 * (b + 1)] = acc[b]
        ctx = [None] * 4

        def mstep(b, h):
            def step():
                a, r = divmod(h, 8)
                o = _dot(row(r, acc[b][8 * a:8 * a + 8]), _tile(wuv_t, VM.index(h) * NC + b))
                ctx[a] = o if ctx[a] is None else ctx[a] + o
            return step

        cur = {}
        done = {}

        def vstep(h, i):
            def step():
                k = VV.index(h)
                if i == 0:
                    xs_ = [bcast_row(a_scr, h, 128 * b) for b in range(NC)]
                    if k >= VLAG:
                        xs_ = [after(done[VV[k - VLAG]], x) for x in xs_]
                    cur["x"] = xs_
                    cur["d"] = 0.0
                p = [cur["x"][b] * wuv_f[(k * 16 + i) * NC + b] for b in range(NC)]
                s = jnp.sum((p[0] + p[1]) + (p[2] + p[3]), axis=-1, keepdims=True)
                cur["d"] = jnp.where(lane == sub + 8 * i, s, cur["d"])
                if i == VGATE:
                    done[h] = jnp.broadcast_to(s, (8, 128))
                if i == 15:
                    ctxv_scr[k] = _rowsum(cur["d"]) * linv[h:h + 1]
            return step

        _interleave([mstep(b, h) for b in range(NC) for h in VM],
                    [vstep(h, i) for h in VV for i in range(16)])
        for a in range(4):
            if ctx[a] is not None:
                ctx_scr[8 * a:8 * a + 8, :] = ctx[a] * linv[8 * a:8 * a + 8]

    def ctx_row(h):
        return ctxv_scr[VV.index(h)] if h in VV else bcast_row(ctx_scr, h)

    def out_first(i, outs):
        cps["wo", i].wait()
        for h in range(WO_SPLIT[i], WO_SPLIT[i + 1]):
            l = ctx_row(h)
            for j in range(NM):
                t = _dot(l, wo_v[128 * h:128 * (h + 1), 128 * j:128 * (j + 1)])
                outs[j] = t if outs[j] is None else outs[j] + t
        if i < NWO - 1:
            relayout_wo(WO_SPLIT[i], WO_SPLIT[i + 1])

    def relayout_wo(h0, h1):
        nv = len(OV)
        assert OV == tuple(range(nv))

        def body_v(h, carry):
            r0 = pl.multiple_of(h * 128, 128)
            for g in range(16):
                wf = wo_v[pl.ds(r0 + 8 * g, 8), :].astype(F32)
                for j in range(NM):
                    wo_f[(h * 16 + g) * NM + j] = wf[:, 128 * j:128 * (j + 1)]
            return carry

        def body_m(h, carry):
            r0 = pl.multiple_of(h * 128, 128)
            for j in range(NM):
                wo_t[(h - nv) * NM + j] = pltpu.bitcast(wo_v[pl.ds(r0, 128), 128 * j:128 * (j + 1)], I32)
            return carry

        if h0 < min(h1, nv):
            lax.fori_loop(h0, min(h1, nv), body_v, 0)
        if max(h0, nv) < h1:
            lax.fori_loop(max(h0, nv), h1, body_m, 0)

    def out_second():
        outs = [None] * NM
        vacc = [None] * NM

        def mstep(h, j):
            def step():
                t = _dot(ctx_row(h), _tile(wo_t, (h - len(OV)) * NM + j))
                outs[j] = t if outs[j] is None else outs[j] + t
            return step

        part = {}

        def prep_o(h, dep):
            src = ctx_row(h)
            return src if dep is None else after(dep, src)

        groups = [OV[k:k + OG] for k in range(0, len(OV), OG)]

        def o_mac(h, g, m):
            grp = next(x for x in groups if h in x)
            for j in range(NM):
                t = m * wo_f[(OV.index(h) * 16 + g) * NM + j]
                part[j] = t if h == grp[0] else part[j] + t
                if h == grp[-1]:
                    vacc[j] = part[j] if vacc[j] is None else vacc[j] + part[j]
            return part[NM - 1]

        _interleave([mstep(h, j) for j in range(NM) for h in OM], column_stream(groups, prep_o, o_mac, OLAG))
        if OV:
            outs = [o + _rowsum(v) for o, v in zip(outs, vacc)]
        return outs

    def ffn_act(xs, mu, rstd):
        acts = [None] * NF
        acc = {}

        def finish(ft):
            g = rstd * (acc[ft, 0] - mu * csgu_scr[ft])
            u = rstd * (acc[ft, 1] - mu * csgu_scr[NF + ft])
            acts[ft] = g * jax.nn.sigmoid(g) * u

        def mstep(ft, which, j):
            def step():
                o = _dot(xs[j], _tile(gu_t, (which * len(GM) + GM.index(ft)) * NM + j))
                acc[ft, which] = o if j == 0 else acc[ft, which] + o
                if j == NM - 1 and which == 1:
                    finish(ft)
            return step

        NTV = 2 * len(GV)
        cur = {}
        vacc = [None] * NTV

        def g_mac(j, g, m):
            for n in range(NTV):
                p = m * gu_f[(j * 16 + g) * NTV + n]
                vacc[n] = p if vacc[n] is None else vacc[n] + p
            return vacc[NTV - 1]

        def prep_g(j, dep):
            return xs[j] if dep is None else after(dep, xs[j])

        mx = []
        for f0 in range(0, len(GM), 2):
            for j in range(NM):
                for ft in GM[f0:f0 + 2]:
                    for which in range(2):
                        mx.append(mstep(ft, which, j))
        _interleave(mx, column_stream([(j,) for j in range(NM)], prep_g, g_mac, GLAG) if GV else [])
        for k, ft in enumerate(GV):
            acc[ft, 0] = _rowsum(vacc[2 * k])
            acc[ft, 1] = _rowsum(vacc[2 * k + 1])
            finish(ft)
        return acts

    def wd_tile(ft, j):
        t = wd_v[128 * ft:min(128 * (ft + 1), F), 128 * j:128 * (j + 1)]
        if ft == NF - 1:
            t = jnp.concatenate([t, jnp.zeros((128 * NF - F, 128), BF16)], axis=0)
        return t

    def ffn_residual(xs, mu, rstd, wr):
        xn = [((v - mu) * rstd).astype(BF16).astype(F32) for v in xs]
        rr = None
        for v, w in zip(xn, wr):
            rr = v * w if rr is None else rr + v * w
        sig = jax.nn.sigmoid(jnp.sum(rr, axis=-1, keepdims=True))
        base = [v + n for v, n in zip(xs, xn)]
        zero = [n * 0.0 for n in xn]
        return base, zero, sig

    cps["x"].wait()
    cps["wr"].wait()
    x_all = jnp.broadcast_to(x_v[...].astype(F32), (8, M))
    wr_all = jnp.broadcast_to(wr_v[...].reshape(1, M).astype(F32), (8, M))
    xs = [x_all[:, 128 * j:128 * (j + 1)] for j in range(NM)]
    wr = [wr_all[:, 128 * j:128 * (j + 1)] for j in range(NM)]
    mu, rstd = stats(xs)
    never = jnp.broadcast_to(rstd, (8, 128)) < 0.0

    def after(dep, v):
        return jnp.where(never, dep, v)

    cps["wq"].wait()
    split_wq()
    qacc = [None] * 4
    for j in range(NM):
        q_part(j, xs[j], qacc, True)
    for a in range(4):
        cs = qacc[a][8:16]
        csq_scr[8 * a:8 * a + 8, :] = cs
        q_scr[16 * a:16 * a + 16, :] = jnp.concatenate([qacc[a][0:8] - mu * cs, zero8], axis=0).astype(BF16)
    cps["wuk"].wait()
    zs = qabs_first(rstd)
    cps["c"].wait()
    scores_first(zs)
    acc, linv = softmax_pv(smax(0), smax(HALF))
    cps["wuv"].wait()
    split_wuv()
    context(acc, linv)
    outs = [None] * NM
    out_first(0, outs)
    cps["wg"].wait()
    transpose_gu(wg_v, 0)
    cps["wu"].wait()
    transpose_gu(wu_v, 1)
    for i in range(1, NWO):
        out_first(i, outs)
    xs = [v + o for v, o in zip(xs, outs)]
    mu, rstd = stats(xs)
    acts = ffn_act(xs, mu, rstd)
    base, zero, sig = ffn_residual(xs, mu, rstd, wr)
    relayout_wo(WO_SPLIT[-2], WO_SPLIT[-1])
    qacc = [None] * 4
    xs = []
    for i in range(NWD):
        cps["wd", i].wait()
        js = range(WD_SPLIT[i], WD_SPLIT[i + 1])
        for j in js:
            y = None
            for ft in range(NF):
                o = _dot(acts[ft], wd_tile(ft, j))
                y = o if y is None else y + o
            xs.append(base[j] + (zero[j] + y * sig))
        for j in js:
            q_part(j, xs[j], qacc, False)

    mu, rstd = stats(xs)
    qs = [qacc[a] - mu * csq_scr[8 * a:8 * a + 8, :] for a in range(4)]
    zs = qabs(qs, rstd)
    m_a = scores(zs, 0)
    m_b = scores(zs, HALF)
    acc, linv = softmax_pv(m_a, m_b)
    context(acc, linv)
    outs = out_second()
    xs = [v + o for v, o in zip(xs, outs)]
    mu, rstd = stats(xs)
    acts = ffn_act(xs, mu, rstd)
    base, zero, sig = ffn_residual(xs, mu, rstd, wr)
    ys = [None] * NM
    yv = [None] * NM
    part = {}
    dgroups = [DV[k:k + DG] for k in range(0, len(DV), DG)]

    def d_mstep(ft, j):
        def step():
            o = _dot(acts[ft], wd_tile(ft, j))
            ys[j] = o if ys[j] is None else ys[j] + o
        return step

    def prep_d(ft, dep):
        return acts[ft] if dep is None else after(dep, acts[ft])

    def d_mac(ft, g, m):
        grp = next(x for x in dgroups if ft in x)
        w = wd_v[128 * ft + 8 * g:128 * ft + 8 * g + 8, :].astype(F32)
        for j in range(NM):
            t = m * w[:, 128 * j:128 * (j + 1)]
            part[j] = t if ft == grp[0] else part[j] + t
            if ft == grp[-1]:
                yv[j] = part[j] if yv[j] is None else yv[j] + part[j]
        return part[NM - 1]

    dm = [ft for ft in range(NF) if ft not in DV]
    _interleave([d_mstep(ft, j) for ft in dm for j in range(NM)], column_stream(dgroups, prep_d, d_mac, DLAG))
    if DV:
        ys = [y + _rowsum(v) for y, v in zip(ys, yv)]
    for j in range(NM):
        xo = base[j] + (zero[j] + ys[j] * sig)
        o_ref[:, 128 * j:128 * (j + 1)] = xo[0:1, :].astype(o_ref.dtype)


@jax.jit
def pallas_interleave_layers__compressed_kv_cla__moe_arch_mod__decode_kernel(
        A_x, A_c_kv, A_w_q, A_w_uk, A_w_uv, A_w_o, B_x, B_w_r, B_w_gate, B_w_up, B_w_down):
    del B_x
    any_spec = pl.BlockSpec(memory_space=pl.ANY)

    def tiles(n):
        return pltpu.VMEM((max(n, 1), 64, 128), I32)

    def vregs(n):
        return pltpu.VMEM((max(n, 1), 8, 128), F32)

    out = pl.pallas_call(
        _kernel,
        out_shape=jax.ShapeDtypeStruct((1, M), BF16),
        in_specs=[any_spec] * 10,
        out_specs=pl.BlockSpec(memory_space=pltpu.VMEM),
        scratch_shapes=[
            pltpu.VMEM((1, M), BF16), pltpu.VMEM((M,), BF16),
            pltpu.VMEM((SK, DC), BF16),
            pltpu.VMEM((M * H, D), BF16), pltpu.VMEM((DC * H, D), BF16), pltpu.VMEM((DC * H, D), BF16),
            pltpu.VMEM((H * D, M), BF16),
            pltpu.VMEM((F, M), BF16), pltpu.VMEM((F, M), BF16), pltpu.VMEM((F, M), BF16),
            tiles(H * NM),
            tiles(len(QM) * NC), vregs(len(QV) * 16 * NC),
            tiles(len(VM) * NC), vregs(len(VV) * 16 * NC),
            tiles(len(OM) * NM), vregs(len(OV) * 16 * NM),
            tiles(NC * NK),
            tiles(2 * len(GM) * NM), vregs(2 * len(GV) * 16 * NM),
            pltpu.VMEM((NK, H, 128), F32), pltpu.VMEM((NC, H, 128), F32), pltpu.VMEM((2 * H, D), BF16),
            pltpu.VMEM((H, DC), F32), pltpu.VMEM((H, D), F32), vregs(len(VV)), pltpu.VMEM((H, D), F32),
            pltpu.VMEM((2 * NF, 8, 128), F32),
            pltpu.SemaphoreType.DMA((8 + NWO + NWD,)),
        ],
        compiler_params=pltpu.CompilerParams(vmem_limit_bytes=110 * 2**20, disable_semaphore_checks=True),
    )(A_x.reshape(1, M), B_w_r, A_c_kv.reshape(SK, DC), A_w_q.reshape(M * H, D),
      A_w_uk.reshape(DC * H, D), A_w_uv.reshape(DC * H, D), A_w_o.reshape(H * D, M),
      B_w_gate.T, B_w_up.T, B_w_down)
    return out.reshape(1, 1, M)
```

```python
import math
import jax
import jax.numpy as jnp
from jax import lax
import jax.experimental.pallas as pl
import jax.experimental.pallas.tpu as pltpu

F32, BF16, I32 = jnp.float32, jnp.bfloat16, jnp.int32
M, H, D, SK, DC, F = 640, 32, 128, 4096, 512, 1728
NM = M // 128
NC = DC // 128
NK = SK // 128
NF = 14
WO_SPLIT = (0, 12, 24, 32)
WD_SPLIT = (0, 2, 4, 5)
NWO = len(WO_SPLIT) - 1
NWD = len(WD_SPLIT) - 1
NN = (((1,), (0,)), ((), ()))
NT = (((1,), (1,)), ((), ()))

QV = tuple(range(12))
VV = tuple(range(11))
OV = tuple(range(12))
GV = tuple(range(9, 14))
VM = tuple(range(11, 32))
OM = tuple(range(12, 32))
DV = tuple(range(4))
DG = 2
DLAG = 10
QG = 3
OG = 3
QLAG = 10
OLAG = 4
GLAG = 5
VLAG = 5
ODELAY = 24
OEARLY = 2
DEARLY = 1
D4V = 12
D4A = 4
DDELAY = 2
DBACK = 0
QDEFER = 4
SU = 2
SLEAD = 2
VGATE = 0
QM = tuple(h for h in range(H) if h not in QV)
GM = tuple(f for f in range(NF) if f not in GV)
NT_V = [(f, w) for f in GV for w in range(2) if (f, w) != (NF - 1, 1)]
assert NF - 1 in GV
assert sorted(VM + VV) == list(range(H)) and sorted(OM + OV) == list(range(H))


GATE = True
FLAGS = None


def _iota(shape, dim):
    return lax.broadcasted_iota(I32, shape, dim)


def _dot(a, b):
    return lax.dot_general(a, b, NN, preferred_element_type=F32)


def _dot_t(a, b):
    return lax.dot_general(a, b, NT, preferred_element_type=F32)


def _tile(ref, i):
    return pltpu.bitcast(ref[i], BF16)


def _words(v):
    return pltpu.bitcast(v.astype(BF16), I32)


def _interleave(mx, vp):
    nm, nv = len(mx), len(vp)
    iv = 0
    for im, step in enumerate(mx):
        step()
        while iv < (im + 1) * nv // nm:
            vp[iv]()
            iv += 1
    while iv < nv:
        vp[iv]()
        iv += 1


def _rowsum(v):
    return jnp.broadcast_to(jnp.sum(v, axis=0, keepdims=True), v.shape)


def _columns(rowvec):
    return jnp.broadcast_to(rowvec[0:1, :], (128, 128)).T


def _kernel(x_hbm, wr_hbm, c_hbm, wq_hbm, wuk_hbm, wuv_hbm, wo_hbm, wg_hbm, wu_hbm, wd_hbm,
            o_ref,
            x_v, wr_v, c_v, wq_v, wuk_v, wuv_v, wo_v, wg_v, wu_v, wd_v,
            wq_t, tmp_t, wuk_t, wuk_f, wuv_t, wuv_f, wo_t, wo_f, c_t, gu_t, gu_f,
            s_scr, z_scr, q_scr, a_scr, ctx_scr, ctxv_scr, csq_scr, csgu_scr, sems):
    pairs = {"wq": (wq_hbm, wq_v), "x": (x_hbm, x_v), "wr": (wr_hbm, wr_v), "wuk": (wuk_hbm, wuk_v),
             "c": (c_hbm, c_v), "wuv": (wuv_hbm, wuv_v), "wg": (wg_hbm, wg_v), "wu": (wu_hbm, wu_v)}
    for i, (h0, h1) in enumerate(zip(WO_SPLIT[:-1], WO_SPLIT[1:])):
        rows = pl.ds(D * h0, D * (h1 - h0))
        pairs["wo", i] = (wo_hbm.at[rows, :], wo_v.at[rows, :])
    for i, (j0, j1) in enumerate(zip(WD_SPLIT[:-1], WD_SPLIT[1:])):
        cols = pl.ds(128 * j0, 128 * (j1 - j0))
        pairs["wd", i] = (wd_hbm.at[:, cols], wd_v.at[:, cols])
    order = ["wq", "x", "wr", "wuk", "c", "wuv", ("wo", 0), "wg", "wu"]
    order += [("wo", i) for i in range(1, NWO)] + [("wd", i) for i in range(NWD)]
    cps = {k: pltpu.make_async_copy(*pairs[k], sems.at[i]) for i, k in enumerate(order)}
    for k in order:
        cps[k].start()

    sub = _iota((8, 128), 0)
    lane = _iota((8, 128), 1)
    zero8 = jnp.zeros((8, 128), F32)
    eye = (_iota((128, 128), 0) == _iota((128, 128), 1)).astype(BF16)

    def row(r, v):
        return jnp.where(sub == r, v, 0.0)

    def bcast_row(ref, r, c0=0):
        return jnp.broadcast_to(ref[r:r + 1, c0:c0 + 128], (8, 128))

    def split_heads(src_v, nrows, store):
        w32 = src_v.bitcast(I32)

        def transpose8(v):
            for k in (4, 2, 1):
                hi = (sub & k) != 0
                w = list(v)
                for a in range(8):
                    if not a & k:
                        w[a] = jnp.where(hi, pltpu.roll(v[a | k], k, 0), v[a])
                        w[a | k] = jnp.where(hi, v[a | k], pltpu.roll(v[a], 8 - k, 0))
                v = w
            return v

        def body(it, carry):
            for e in range(SU):
                g = it * SU + e
                base = pl.multiple_of(g * 256, 256)
                blk = lax.shift_right_logical(g, 3)
                rows = pl.ds(pl.multiple_of((g & 7) * 8, 8), 8)
                for hh in range(2):
                    ev = transpose8([w32[pl.ds(base + 32 * i + 8 * hh, 8), :] for i in range(8)])
                    od = transpose8([w32[pl.ds(base + 32 * i + 16 + 8 * hh, 8), :] for i in range(8)])
                    for j in range(8):
                        a, b = ev[j], od[j]
                        h = 16 * hh + 2 * j
                        store(h, blk, (a & 0xFFFF) | (b << 16), rows)
                        store(h + 1, blk, lax.shift_right_logical(a, 16) | (b & -65536), rows)
            return carry

        lax.fori_loop(0, nrows // (16 * SU), body, 0)

    def split_wq():
        def store(h, blk, w, rows):
            wq_t[h * NM + blk, rows, :] = w
        split_heads(wq_v, M, store)

    def split_natural(src_v):
        def store(h, blk, w, rows):
            tmp_t[h * NC + blk, rows, :] = w
        split_heads(src_v, DC, store)

    def split_wuv():
        def store(h, blk, w, rows):
            if h in VM:
                wuv_t[sorted(VM).index(h) * NC + blk, rows, :] = w
            else:
                tmp_t[VV.index(h) * NC + blk, rows, :] = w
        split_heads(wuv_v, DC, store)

        def body(b, carry):
            for k in range(len(VV)):
                t = _dot_t(eye, _tile(tmp_t, k * NC + b))
                for i in range(16):
                    wuv_f[(k * 16 + i) * NC + b] = t[8 * i:8 * i + 8]
            return carry

        lax.fori_loop(0, NC, body, 0)

    def transpose_gu(src_v, which):
        lhs = jnp.concatenate([eye, jnp.ones((16, 128), BF16)], axis=0)
        fts = list(range(NF - 1)) + ([NF - 1] if which == 1 else [])

        def body(j, carry):
            cols = pl.ds(pl.multiple_of(j * 128, 128), 128)
            css = []
            for k, ft in enumerate(fts):
                if ft < NF - 1:
                    t = src_v[128 * ft:128 * (ft + 1), cols]
                    n = NT_V.index((ft, which)) if ft in GV else None
                else:
                    t = jnp.concatenate([wg_v[128 * ft:F, cols], wu_v[128 * ft:F, cols]], axis=0)
                    n = NT_V.index((ft, 0))
                o = _dot_t(lhs, t)
                if n is None:
                    gu_t[(which * len(GM) + GM.index(ft)) * NM + j] = _words(o[0:128])
                else:
                    for g in range(16):
                        gu_f[(j * 16 + g) * len(NT_V) + n] = o[8 * g:8 * g + 8]
                css.append(carry[k] + o[128:136])
            return tuple(css)

        css = lax.fori_loop(0, NM, body, (zero8,) * len(fts))
        for k, ft in enumerate(fts):
            csgu_scr[which * NF + ft] = css[k]

    class ColumnStream:
        def __init__(self, groups, prep, mac, lag):
            self.groups, self.prep, self.mac, self.lag = groups, prep, mac, lag
            self.cols = {}

        def start(self, i, dep=None):
            if i < len(self.groups) and self.groups[i][0] not in self.cols:
                for key in self.groups[i]:
                    v = self.prep(key)
                    self.cols[key] = _columns(v if dep is None else after(dep, v))

        def steps(self):
            def make(i, g):
                def step():
                    if i == 0 and g == 0:
                        self.start(0)
                        self.start(1)
                    last = None
                    for key in self.groups[i]:
                        last = self.mac(key, g, self.cols[key][8 * g:8 * g + 8])
                    if g == self.lag:
                        self.start(i + 2, last)
                return step

            return [make(i, g) for i in range(len(self.groups)) for g in range(16)]

    def stats(xs):
        tot = xs[0]
        for v in xs[1:]:
            tot = tot + v
        mu = jnp.sum(tot, axis=-1, keepdims=True) * (1.0 / M)
        sq = None
        for v in xs:
            d = v - mu
            sq = d * d if sq is None else sq + d * d
        var = jnp.sum(sq, axis=-1, keepdims=True) * (1.0 / M)
        return mu, lax.rsqrt(var + 1e-5)

    ones_rows = [row(r, 1.0) for r in range(8)]

    def q_part(j, xj, acc, first, heads):
        lhs = []
        for r in range(8):
            l = row(r, xj)
            if first:
                l = jnp.concatenate([l, ones_rows[r]], axis=0)
            lhs.append(l)
        for h in heads:
            o = _dot(lhs[h % 8], _tile(wq_t, h * NM + j))
            acc[h // 8] = o if acc[h // 8] is None else acc[h // 8] + o

    QSCALE = D ** -0.5 * math.log2(math.e)

    def qabs(qs, rstd):
        scale = rstd * QSCALE
        z = [[zero8] * 4 for _ in range(NC)]

        def mstep(b, h):
            def step():
                o = _dot(qs[h // 8], _tile(wuk_t, QM.index(h) * NC + b))
                z[b][h // 8] = jnp.where(sub == h % 8, o, z[b][h // 8])
            return step

        vqacc = {}
        groups = [QV[k:k + QG] for k in range(0, len(QV), QG)]

        def prep_q(h):
            return _rowsum(row(h % 8, qs[h // 8]))

        def q_mac(h, g, m):
            for b in range(NC):
                p = m * wuk_f[(QV.index(h) * 16 + g) * NC + b]
                vqacc[h, b] = p if g == 0 else vqacc[h, b] + p
                if g == 15:
                    z[b][h // 8] = jnp.where(sub == h % 8, _rowsum(vqacc[h, b]), z[b][h // 8])
            return vqacc[h, NC - 1]

        _interleave([mstep(b, h) for b in range(NC) for h in QM],
                    ColumnStream(groups, prep_q, q_mac, QLAG).steps())
        return [jnp.concatenate([v * scale for v in z[b]], axis=0).astype(BF16) for b in range(NC)]

    def qabs_first(rstd):
        split_natural(wuk_v)
        scale = rstd * QSCALE

        def body(b, carry):
            z = [zero8] * 4
            for h in range(H):
                a = h // 8
                qb = q_scr[16 * a:16 * a + 16, :]
                lhs = jnp.concatenate([eye, qb], axis=0)
                o = _dot_t(lhs, _tile(tmp_t, h * NC + b))
                if h in QM:
                    wuk_t[QM.index(h) * NC + b] = _words(o[0:128])
                else:
                    for g in range(16):
                        wuk_f[(QV.index(h) * 16 + g) * NC + b] = o[8 * g:8 * g + 8]
                z[a] = jnp.where(sub == h % 8, o[128:136], z[a])
            z_scr[b] = jnp.concatenate([v * scale for v in z], axis=0)
            return carry

        lax.fori_loop(0, NC, body, 0)
        return [z_scr[b].astype(BF16) for b in range(NC)]

    def scores_first(zs):
        lhs = [jnp.concatenate([eye, zs[b]], axis=0) for b in range(NC)]
        U = 4

        def body(g, carry):
            for i in range(U):
                t = g * U + i
                r0 = pl.multiple_of(t * 128, 128)
                s = None
                for b in range(NC):
                    o = _dot_t(lhs[b], c_v[pl.ds(r0, 128), 128 * b:128 * (b + 1)])
                    c_t[b * NK + t] = _words(o[0:128])
                    s = o[128:160] if s is None else s + o[128:160]
                s_scr[t] = s
            return carry

        lax.fori_loop(0, NK // U, body, 0)

    HALF = NK // 2

    def scores(zs, t0):
        mx = None
        acc = {}

        def tile(t, b):
            o = _dot(zs[b], _tile(c_t, b * NK + t))
            acc[t] = o if b == 0 else acc[t] + o

        groups = [list(range(g0, g0 + 4)) for g0 in range(t0, t0 + HALF, 4)]
        if t0 == 0:
            for b in range(NC - 1):
                for grp in groups[:SLEAD]:
                    for t in grp:
                        tile(t, b)
            for grp in groups[:SLEAD]:
                for t in grp:
                    tile(t, NC - 1)
        for k, grp in enumerate(groups):
            if t0 != 0 or k >= SLEAD:
                for b in range(NC):
                    for t in grp:
                        tile(t, b)
            for t in grp:
                s_scr[t] = acc[t]
                mx = acc[t] if mx is None else jnp.maximum(mx, acc[t])
        return jnp.max(mx, axis=-1, keepdims=True)

    def smax(t0):
        mx = None
        for t in range(t0, t0 + HALF):
            v = s_scr[t]
            mx = v if mx is None else jnp.maximum(mx, v)
        return jnp.max(mx, axis=-1, keepdims=True)

    def softmax_pv(m_a, m_b):
        m = jnp.maximum(m_a, m_b)
        alpha = jnp.exp2(m_a - m)

        def cv(t, b):
            return c_v[128 * t:128 * (t + 1), 128 * b:128 * (b + 1)]

        acc = [None] * NC
        lsum = None
        for t in range(HALF):
            p = jnp.exp2(s_scr[t] - m_a)
            lsum = p if lsum is None else lsum + p
            pb = p.astype(BF16)
            for b in range(NC):
                o = _dot(pb, cv(t, b))
                acc[b] = o if acc[b] is None else acc[b] + o
        lsum = lsum * alpha
        acc = [v * alpha for v in acc]
        for t in range(HALF, HALF + 8):
            p = jnp.exp2(s_scr[t] - m)
            lsum = lsum + p
            pb = p.astype(BF16)
            for b in range(NC):
                acc[b] = acc[b] + _dot(pb, cv(t, b))
        pbs = {}
        for b in range(NC):
            for t in range(HALF + 8, NK):
                if b == 0:
                    p = jnp.exp2(s_scr[t] - m)
                    lsum = lsum + p
                    pbs[t] = p.astype(BF16)
                acc[b] = acc[b] + _dot(pbs[t], cv(t, b))
        linv = 1.0 / jnp.sum(lsum, axis=-1, keepdims=True)
        return acc, linv

    def context(acc, linv, nxt=None):
        for b in range(NC):
            a_scr[:, 128 * b:128 * (b + 1)] = acc[b]
        ctx = [None] * 4

        def mstep(b, h):
            def step():
                a, r = divmod(h, 8)
                o = _dot(row(r, acc[b][8 * a:8 * a + 8]), _tile(wuv_t, sorted(VM).index(h) * NC + b))
                ctx[a] = o if ctx[a] is None else ctx[a] + o
            return step

        cur = {}
        done = {}

        def vstep(h, i):
            def step():
                k = VV.index(h)
                if i == 0:
                    xs_ = [bcast_row(a_scr, h, 128 * b) for b in range(NC)]
                    if k >= VLAG:
                        xs_ = [after(done[VV[k - VLAG]], x) for x in xs_]
                    cur["x"] = xs_
                    cur["d"] = 0.0
                p = [cur["x"][b] * wuv_f[(k * 16 + i) * NC + b] for b in range(NC)]
                s = jnp.sum((p[0] + p[1]) + (p[2] + p[3]), axis=-1, keepdims=True)
                cur["d"] = jnp.where(lane == sub + 8 * i, s, cur["d"])
                if i == VGATE:
                    done[h] = jnp.broadcast_to(s, (8, 128))
                if i == 15:
                    ctxv_scr[k] = _rowsum(cur["d"]) * linv[h:h + 1]
                if nxt is not None and i == ODELAY % 16:
                    for gi, grp in enumerate(nxt.groups[:OEARLY]):
                        if all(x in VV and VV.index(x) <= k - 1 - ODELAY // 16 for x in grp):
                            nxt.start(gi)
            return step

        _interleave([mstep(b, h) for b in range(NC) for h in VM],
                    [vstep(h, i) for h in VV for i in range(16)])
        for a in range(4):
            if ctx[a] is not None:
                ctx_scr[8 * a:8 * a + 8, :] = ctx[a] * linv[8 * a:8 * a + 8]

    def ctx_row(h):
        return ctxv_scr[VV.index(h)] if h in VV else bcast_row(ctx_scr, h)

    def out_first(i, outs):
        cps["wo", i].wait()
        for h in range(WO_SPLIT[i], WO_SPLIT[i + 1]):
            l = ctx_row(h)
            for j in range(NM):
                t = _dot(l, wo_v[128 * h:128 * (h + 1), 128 * j:128 * (j + 1)])
                outs[j] = t if outs[j] is None else outs[j] + t
        if i < NWO - 1:
            relayout_wo(WO_SPLIT[i], WO_SPLIT[i + 1])

    def relayout_wo(h0, h1):
        nv = len(OV)
        assert OV == tuple(range(nv))

        def body_v(h, carry):
            r0 = pl.multiple_of(h * 128, 128)
            for g in range(16):
                wf = wo_v[pl.ds(r0 + 8 * g, 8), :].astype(F32)
                for j in range(NM):
                    wo_f[(h * 16 + g) * NM + j] = wf[:, 128 * j:128 * (j + 1)]
            return carry

        def body_m(h, carry):
            r0 = pl.multiple_of(h * 128, 128)
            for j in range(NM):
                wo_t[(h - nv) * NM + j] = pltpu.bitcast(wo_v[pl.ds(r0, 128), 128 * j:128 * (j + 1)], I32)
            return carry

        if h0 < min(h1, nv):
            lax.fori_loop(h0, min(h1, nv), body_v, 0)
        if max(h0, nv) < h1:
            lax.fori_loop(max(h0, nv), h1, body_m, 0)

    def out_second():
        outs = [None] * NM
        vacc = [None] * NM

        def mstep(h, j):
            def step():
                t = _dot(ctx_row(h), _tile(wo_t, (h - len(OV)) * NM + j))
                outs[j] = t if outs[j] is None else outs[j] + t
            return step

        part = {}
        groups = [OV[k:k + OG] for k in range(0, len(OV), OG)]

        def o_mac(h, g, m):
            grp = next(x for x in groups if h in x)
            for j in range(NM):
                t = m * wo_f[(OV.index(h) * 16 + g) * NM + j]
                part[j] = t if h == grp[0] else part[j] + t
                if h == grp[-1]:
                    vacc[j] = part[j] if vacc[j] is None else vacc[j] + part[j]
            return part[NM - 1]

        stream = ColumnStream(groups, ctx_row, o_mac, OLAG)

        def run():
            _interleave([mstep(h, j) for j in range(NM) for h in OM], stream.steps())
            return [o + _rowsum(v) for o, v in zip(outs, vacc)]

        return stream, run

    def ffn_act(xs, mu, rstd, acts, nxt=None):
        acc = {}

        def finish(ft):
            g = rstd * (acc[ft, 0] - mu * csgu_scr[ft])
            u = rstd * (acc[ft, 1] - mu * csgu_scr[NF + ft])
            acts[ft] = g * jax.nn.sigmoid(g) * u

        def mstep(ft, which, j):
            def step():
                o = _dot(xs[j], _tile(gu_t, (which * len(GM) + GM.index(ft)) * NM + j))
                acc[ft, which] = o if j == 0 else acc[ft, which] + o
                if j == NM - 1 and which == 1:
                    finish(ft)
                if nxt is not None and j == DDELAY and which == 0:
                    for grp_i, grp in enumerate(nxt.groups[:DEARLY]):
                        if all(acts[x] is not None for x in grp) and grp[-1] < ft // 2 * 2 - DBACK:
                            nxt.start(grp_i)
            return step

        NTV = len(NT_V)
        cur = {}
        vacc = [None] * NTV

        def g_mac(j, g, m):
            for n in range(NTV):
                p = m * gu_f[(j * 16 + g) * NTV + n]
                vacc[n] = p if vacc[n] is None else vacc[n] + p
            return vacc[NTV - 1]

        mx = []
        for f0 in range(0, len(GM), 2):
            for j in range(NM):
                for ft in GM[f0:f0 + 2]:
                    for which in range(2):
                        mx.append(mstep(ft, which, j))
        _interleave(mx, ColumnStream([(j,) for j in range(NM)], lambda j: xs[j], g_mac, GLAG).steps())
        for ft in GV[::-1]:
            if ft < NF - 1:
                acc[ft, 0] = _rowsum(vacc[NT_V.index((ft, 0))])
                acc[ft, 1] = _rowsum(vacc[NT_V.index((ft, 1))])
                finish(ft)
            else:
                g = rstd * (_rowsum(vacc[NT_V.index((ft, 0))]) - mu * csgu_scr[NF + ft])
                acts[ft] = g * jax.nn.sigmoid(g) * pltpu.roll(g, 64, 1)
        return acts

    def down(act, ft, j):
        rows = min(128, F - 128 * ft)
        return _dot(act[:, 0:rows], wd_v[128 * ft:128 * ft + rows, 128 * j:128 * (j + 1)])

    def ffn_residual(xs, mu, rstd, wr):
        xn = [((v - mu) * rstd).astype(BF16).astype(F32) for v in xs]
        rr = None
        for v, w in zip(xn, wr):
            rr = v * w if rr is None else rr + v * w
        sig = jax.nn.sigmoid(jnp.sum(rr, axis=-1, keepdims=True))
        base = [v + n for v, n in zip(xs, xn)]
        zero = [n * 0.0 for n in xn]
        return base, zero, sig

    cps["x"].wait()
    cps["wr"].wait()
    x_all = jnp.broadcast_to(x_v[...].astype(F32), (8, M))
    wr_all = jnp.broadcast_to(wr_v[...].reshape(1, M).astype(F32), (8, M))
    xs = [x_all[:, 128 * j:128 * (j + 1)] for j in range(NM)]
    wr = [wr_all[:, 128 * j:128 * (j + 1)] for j in range(NM)]
    mu, rstd = stats(xs)
    never = jnp.broadcast_to(rstd, (8, 128)) < 0.0

    def after(dep, v):
        return jnp.where(never, dep, v) if GATE else v

    cps["wq"].wait()
    split_wq()
    qacc = [None] * 4
    for j in range(NM):
        q_part(j, xs[j], qacc, True, range(H))
    for a in range(4):
        cs = qacc[a][8:16]
        csq_scr[8 * a:8 * a + 8, :] = cs
        q_scr[16 * a:16 * a + 16, :] = jnp.concatenate([qacc[a][0:8] - mu * cs, zero8], axis=0).astype(BF16)
    cps["wuk"].wait()
    zs = qabs_first(rstd)
    cps["c"].wait()
    scores_first(zs)
    acc, linv = softmax_pv(smax(0), smax(HALF))
    cps["wuv"].wait()
    split_wuv()
    context(acc, linv)
    outs = [None] * NM
    out_first(0, outs)
    cps["wg"].wait()
    transpose_gu(wg_v, 0)
    cps["wu"].wait()
    transpose_gu(wu_v, 1)
    for i in range(1, NWO):
        out_first(i, outs)
    xs = [v + o for v, o in zip(xs, outs)]
    mu, rstd = stats(xs)
    acts = ffn_act(xs, mu, rstd, [None] * NF)
    base, zero, sig = ffn_residual(xs, mu, rstd, wr)
    relayout_wo(WO_SPLIT[-2], WO_SPLIT[-1])
    qacc = [None] * 4
    xs = []


    def down_col(j, fts, y=None):
        for ft in fts:
            o = down(acts[ft], ft, j)
            y = o if y is None else y + o
        return y

    for i in range(NWD - 1):
        if i == NWD - 2:
            acol = {ft: _columns(acts[ft]) for ft in range(D4V)}
        cps["wd", i].wait()
        js = range(WD_SPLIT[i], WD_SPLIT[i + 1])
        for j in js:
            xs.append(base[j] + (zero[j] + down_col(j, range(NF)) * sig))
        for j in js:
            q_part(j, xs[j], qacc, False, range(H) if j < NM - 2 else range(H - QDEFER))
    j = NM - 1
    cps["wd", NWD - 1].wait()
    y = down_col(j, range(D4V, NF))
    q_part(j - 1, xs[j - 1], qacc, False, range(H - QDEFER, H))
    if D4V:
        pv = [None] * D4A
        for ft in range(D4V):
            for g in range(16):
                r0 = 128 * ft + 8 * g
                t = acol[ft][8 * g:8 * g + 8] * wd_v[r0:r0 + 8, 128 * j:128 * (j + 1)].astype(F32)
                k = g % D4A
                pv[k] = t if pv[k] is None else pv[k] + t
        tot = pv[0]
        for v in pv[1:]:
            tot = tot + v
        y = _rowsum(tot) if y is None else y + _rowsum(tot)
    xs.append(base[j] + (zero[j] + y * sig))
    q_part(j, xs[j], qacc, False, range(H))

    mu, rstd = stats(xs)
    qs = [qacc[a] - mu * csq_scr[8 * a:8 * a + 8, :] for a in range(4)]
    zs = qabs(qs, rstd)
    m_a = scores(zs, 0)
    m_b = scores(zs, HALF)
    acc, linv = softmax_pv(m_a, m_b)
    o_stream, o_run = out_second()
    context(acc, linv, o_stream)
    outs = o_run()
    xs = [v + o for v, o in zip(xs, outs)]
    mu, rstd = stats(xs)
    acts = [None] * NF
    ys = [None] * NM
    yv = [None] * NM
    part = {}
    dgroups = [DV[k:k + DG] for k in range(0, len(DV), DG)]

    def d_mstep(ft, j):
        def step():
            o = down(acts[ft], ft, j)
            ys[j] = o if ys[j] is None else ys[j] + o
        return step

    def d_mac(ft, g, m):
        grp = next(x for x in dgroups if ft in x)
        w = wd_v[128 * ft + 8 * g:128 * ft + 8 * g + 8, :].astype(F32)
        for j in range(NM):
            t = m * w[:, 128 * j:128 * (j + 1)]
            part[j] = t if ft == grp[0] else part[j] + t
            if ft == grp[-1]:
                yv[j] = part[j] if yv[j] is None else yv[j] + part[j]
        return part[NM - 1]

    d_stream = ColumnStream(dgroups, lambda ft: acts[ft], d_mac, DLAG)
    ffn_act(xs, mu, rstd, acts, d_stream)
    base, zero, sig = ffn_residual(xs, mu, rstd, wr)
    dm = [ft for ft in range(NF) if ft not in DV]
    _interleave([d_mstep(ft, j) for ft in dm for j in range(NM)], d_stream.steps())
    if DV:
        ys = [y + _rowsum(v) for y, v in zip(ys, yv)]
    for j in range(NM):
        xo = base[j] + (zero[j] + ys[j] * sig)
        o_ref[:, 128 * j:128 * (j + 1)] = xo[0:1, :].astype(o_ref.dtype)


@jax.jit
def pallas_interleave_layers__compressed_kv_cla__moe_arch_mod__decode_kernel(
        A_x, A_c_kv, A_w_q, A_w_uk, A_w_uv, A_w_o, B_x, B_w_r, B_w_gate, B_w_up, B_w_down):
    del B_x
    any_spec = pl.BlockSpec(memory_space=pl.ANY)

    def tiles(n):
        return pltpu.VMEM((max(n, 1), 64, 128), I32)

    def vregs(n):
        return pltpu.VMEM((max(n, 1), 8, 128), F32)

    out = pl.pallas_call(
        _kernel,
        out_shape=jax.ShapeDtypeStruct((1, M), BF16),
        in_specs=[any_spec] * 10,
        out_specs=pl.BlockSpec(memory_space=pltpu.VMEM),
        scratch_shapes=[
            pltpu.VMEM((1, M), BF16), pltpu.VMEM((M,), BF16),
            pltpu.VMEM((SK, DC), BF16),
            pltpu.VMEM((M * H, D), BF16), pltpu.VMEM((DC * H, D), BF16), pltpu.VMEM((DC * H, D), BF16),
            pltpu.VMEM((H * D, M), BF16),
            pltpu.VMEM((F, M), BF16), pltpu.VMEM((F, M), BF16), pltpu.VMEM((F, M), BF16),
            tiles(H * NM), tiles(H * NC),
            tiles(len(QM) * NC), vregs(len(QV) * 16 * NC),
            tiles(len(VM) * NC), vregs(len(VV) * 16 * NC),
            tiles(len(OM) * NM), vregs(len(OV) * 16 * NM),
            tiles(NC * NK),
            tiles(2 * len(GM) * NM), vregs(len(NT_V) * 16 * NM),
            pltpu.VMEM((NK, H, 128), F32), pltpu.VMEM((NC, H, 128), F32), pltpu.VMEM((2 * H, D), BF16),
            pltpu.VMEM((H, DC), F32), pltpu.VMEM((H, D), F32), vregs(len(VV)), pltpu.VMEM((H, D), F32),
            pltpu.VMEM((2 * NF, 8, 128), F32),
            pltpu.SemaphoreType.DMA((8 + NWO + NWD,)),
        ],
        compiler_params=pltpu.CompilerParams(vmem_limit_bytes=110 * 2**20, disable_semaphore_checks=True, flags=FLAGS),
    )(A_x.reshape(1, M), B_w_r, A_c_kv.reshape(SK, DC), A_w_q.reshape(M * H, D),
      A_w_uk.reshape(DC * H, D), A_w_uv.reshape(DC * H, D), A_w_o.reshape(H * D, M),
      B_w_gate.T, B_w_up.T, B_w_down)
    return out.reshape(1, 1, M)
```

```python
import math

import jax
import jax.numpy as jnp
from jax import lax
import jax.experimental.pallas as pl
import jax.experimental.pallas.tpu as pltpu

F32, BF16, I32 = jnp.float32, jnp.bfloat16, jnp.int32
M, H, D, SK, DC, F = 640, 32, 128, 4096, 512, 1728
NM = M // 128
NC = DC // 128
NK = SK // 128
NF = 14
WO_SPLIT = (0, 12, 24, 32)
WD_SPLIT = (0, 2, 4, 5)
NWO = len(WO_SPLIT) - 1
NWD = len(WD_SPLIT) - 1
NN = (((1,), (0,)), ((), ()))
NT = (((1,), (1,)), ((), ()))

QV = tuple(range(12))
VV = tuple(range(11))
OV = tuple(range(12))
GV = tuple(range(9, NF))
DV = tuple(range(4))
D4V = 12
QM = tuple(h for h in range(H) if h not in QV)
VM = tuple(h for h in range(H) if h not in VV)
OM = tuple(h for h in range(H) if h not in OV)
GM = tuple(f for f in range(NF) if f not in GV)
GV_TILES = [(f, w) for f in GV for w in range(2) if (f, w) != (NF - 1, 1)]
QG, OG, DG = 3, 3, 2
QLAG, OLAG, GLAG, DLAG, VLAG = 10, 4, 5, 6, 4
SLEAD, QDEFER, DEARLY, D4A = 3, 4, 2, 4
assert NF - 1 in GV and OV == tuple(range(len(OV)))


def _iota(shape, dim):
    return lax.broadcasted_iota(I32, shape, dim)


def _dot(a, b):
    return lax.dot_general(a, b, NN, preferred_element_type=F32)


def _dot_t(a, b):
    return lax.dot_general(a, b, NT, preferred_element_type=F32)


def _tile(ref, i):
    return pltpu.bitcast(ref[i], BF16)


def _words(v):
    return pltpu.bitcast(v.astype(BF16), I32)


def _interleave(mx, vp):
    nm, nv = len(mx), len(vp)
    iv = 0
    for im, step in enumerate(mx):
        step()
        while iv < (im + 1) * nv // nm:
            vp[iv]()
            iv += 1
    while iv < nv:
        vp[iv]()
        iv += 1


def _rowsum(v):
    return jnp.broadcast_to(jnp.sum(v, axis=0, keepdims=True), v.shape)


def _columns(rowvec):
    return jnp.broadcast_to(rowvec[0:1, :], (128, 128)).T


def _kernel(x_hbm, wr_hbm, c_hbm, wq_hbm, wuk_hbm, wuv_hbm, wo_hbm, wg_hbm, wu_hbm, wd_hbm,
            o_ref,
            x_v, wr_v, c_v, wq_v, wuk_v, wuv_v, wo_v, wg_v, wu_v, wd_v,
            wq_t, tmp_t, wuk_t, wuk_f, wuv_t, wuv_f, wo_t, wo_f, c_t, gu_t, gu_f,
            s_scr, z_scr, q_scr, a_scr, ctx_scr, ctxv_scr, csq_scr, csgu_scr, sems):
    pairs = {"wq": (wq_hbm, wq_v), "x": (x_hbm, x_v), "wr": (wr_hbm, wr_v), "wuk": (wuk_hbm, wuk_v),
             "c": (c_hbm, c_v), "wuv": (wuv_hbm, wuv_v), "wg": (wg_hbm, wg_v), "wu": (wu_hbm, wu_v)}
    for i, (h0, h1) in enumerate(zip(WO_SPLIT[:-1], WO_SPLIT[1:])):
        rows = pl.ds(D * h0, D * (h1 - h0))
        pairs["wo", i] = (wo_hbm.at[rows, :], wo_v.at[rows, :])
    for i, (j0, j1) in enumerate(zip(WD_SPLIT[:-1], WD_SPLIT[1:])):
        cols = pl.ds(128 * j0, 128 * (j1 - j0))
        pairs["wd", i] = (wd_hbm.at[:, cols], wd_v.at[:, cols])
    order = ["wq", "x", "wr", "wuk", "c", "wuv", ("wo", 0), "wg", "wu"]
    order += [("wo", i) for i in range(1, NWO)] + [("wd", i) for i in range(NWD)]
    cps = {k: pltpu.make_async_copy(*pairs[k], sems.at[i]) for i, k in enumerate(order)}
    for k in order:
        cps[k].start()

    sub = _iota((8, 128), 0)
    lane = _iota((8, 128), 1)
    zero8 = jnp.zeros((8, 128), F32)
    eye = (_iota((128, 128), 0) == _iota((128, 128), 1)).astype(BF16)

    def row(r, v):
        return jnp.where(sub == r, v, 0.0)

    def bcast_row(ref, r, c0=0):
        return jnp.broadcast_to(ref[r:r + 1, c0:c0 + 128], (8, 128))

    def split_heads(src_v, nrows, store):
        w32 = src_v.bitcast(I32)

        def transpose8(v):
            for k in (4, 2, 1):
                hi = (sub & k) != 0
                w = list(v)
                for a in range(8):
                    if not a & k:
                        w[a] = jnp.where(hi, pltpu.roll(v[a | k], k, 0), v[a])
                        w[a | k] = jnp.where(hi, v[a | k], pltpu.roll(v[a], 8 - k, 0))
                v = w
            return v

        def body(g, carry):
            base = pl.multiple_of(g * 256, 256)
            blk = lax.shift_right_logical(g, 3)
            rows = pl.ds(pl.multiple_of((g & 7) * 8, 8), 8)
            for hh in range(2):
                ev = transpose8([w32[pl.ds(base + 32 * i + 8 * hh, 8), :] for i in range(8)])
                od = transpose8([w32[pl.ds(base + 32 * i + 16 + 8 * hh, 8), :] for i in range(8)])
                for j in range(8):
                    a, b = ev[j], od[j]
                    h = 16 * hh + 2 * j
                    store(h, blk, (a & 0xFFFF) | (b << 16), rows)
                    store(h + 1, blk, lax.shift_right_logical(a, 16) | (b & -65536), rows)
            return carry

        lax.fori_loop(0, nrows // 16, body, 0)

    def split_wq():
        def store(h, blk, w, rows):
            wq_t[h * NM + blk, rows, :] = w
        split_heads(wq_v, M, store)

    def split_natural(src_v):
        def store(h, blk, w, rows):
            tmp_t[h * NC + blk, rows, :] = w
        split_heads(src_v, DC, store)

    def split_wuv():
        def store(h, blk, w, rows):
            if h in VM:
                wuv_t[VM.index(h) * NC + blk, rows, :] = w
            else:
                tmp_t[VV.index(h) * NC + blk, rows, :] = w
        split_heads(wuv_v, DC, store)

        def body(b, carry):
            for k in range(len(VV)):
                t = _dot_t(eye, _tile(tmp_t, k * NC + b))
                for i in range(16):
                    wuv_f[(k * 16 + i) * NC + b] = t[8 * i:8 * i + 8]
            return carry

        lax.fori_loop(0, NC, body, 0)

    def transpose_gu(src_v, which):
        lhs = jnp.concatenate([eye, jnp.ones((16, 128), BF16)], axis=0)
        fts = list(range(NF - 1)) + ([NF - 1] if which == 1 else [])

        def body(j, carry):
            cols = pl.ds(pl.multiple_of(j * 128, 128), 128)
            css = []
            for k, ft in enumerate(fts):
                if ft < NF - 1:
                    t = src_v[128 * ft:128 * (ft + 1), cols]
                    n = GV_TILES.index((ft, which)) if ft in GV else None
                else:
                    t = jnp.concatenate([wg_v[128 * ft:F, cols], wu_v[128 * ft:F, cols]], axis=0)
                    n = GV_TILES.index((ft, 0))
                o = _dot_t(lhs, t)
                if n is None:
                    gu_t[(which * len(GM) + GM.index(ft)) * NM + j] = _words(o[0:128])
                else:
                    for g in range(16):
                        gu_f[(j * 16 + g) * len(GV_TILES) + n] = o[8 * g:8 * g + 8]
                css.append(carry[k] + o[128:136])
            return tuple(css)

        css = lax.fori_loop(0, NM, body, (zero8,) * len(fts))
        for k, ft in enumerate(fts):
            csgu_scr[which * NF + ft] = css[k]

    class Columns:
        def __init__(self, groups, prep, mac, lag):
            self.groups, self.prep, self.mac, self.lag = groups, prep, mac, lag
            self.cols = {}

        def start(self, i, dep=None):
            if i < len(self.groups) and self.groups[i][0] not in self.cols:
                for key in self.groups[i]:
                    v = self.prep(key)
                    self.cols[key] = _columns(v if dep is None else after(dep, v))

        def steps(self):
            def make(i, g):
                def step():
                    if i == 0 and g == 0:
                        self.start(0)
                        self.start(1)
                    last = None
                    for key in self.groups[i]:
                        last = self.mac(key, g, self.cols[key][8 * g:8 * g + 8])
                    if g == self.lag:
                        self.start(i + 2, last)
                return step

            return [make(i, g) for i in range(len(self.groups)) for g in range(16)]

    def stats(xs):
        tot = xs[0]
        for v in xs[1:]:
            tot = tot + v
        mu = jnp.sum(tot, axis=-1, keepdims=True) * (1.0 / M)
        sq = None
        for v in xs:
            d = v - mu
            sq = d * d if sq is None else sq + d * d
        var = jnp.sum(sq, axis=-1, keepdims=True) * (1.0 / M)
        return mu, lax.rsqrt(var + 1e-5)

    ones_rows = [row(r, 1.0) for r in range(8)]

    def q_part(j, xj, acc, first, heads):
        lhs = []
        for r in range(8):
            l = row(r, xj)
            if first:
                l = jnp.concatenate([l, ones_rows[r]], axis=0)
            lhs.append(l)
        for h in heads:
            o = _dot(lhs[h % 8], _tile(wq_t, h * NM + j))
            acc[h // 8] = o if acc[h // 8] is None else acc[h // 8] + o

    QSCALE = D ** -0.5 * math.log2(math.e)

    def qabs(qs, rstd):
        scale = rstd * QSCALE
        z = [[zero8] * 4 for _ in range(NC)]

        def mstep(b, h):
            def step():
                o = _dot(qs[h // 8], _tile(wuk_t, QM.index(h) * NC + b))
                z[b][h // 8] = jnp.where(sub == h % 8, o, z[b][h // 8])
            return step

        vqacc = {}
        groups = [QV[k:k + QG] for k in range(0, len(QV), QG)]

        def prep_q(h):
            return _rowsum(row(h % 8, qs[h // 8]))

        def q_mac(h, g, m):
            for b in range(NC):
                p = m * wuk_f[(QV.index(h) * 16 + g) * NC + b]
                vqacc[h, b] = p if g == 0 else vqacc[h, b] + p
                if g == 15:
                    z[b][h // 8] = jnp.where(sub == h % 8, _rowsum(vqacc[h, b]), z[b][h // 8])
            return vqacc[h, NC - 1]

        _interleave([mstep(b, h) for b in range(NC) for h in QM],
                    Columns(groups, prep_q, q_mac, QLAG).steps())
        return [jnp.concatenate([v * scale for v in z[b]], axis=0).astype(BF16) for b in range(NC)]

    def qabs_first(rstd):
        split_natural(wuk_v)
        scale = rstd * QSCALE

        def body(b, carry):
            z = [zero8] * 4
            for h in range(H):
                a = h // 8
                qb = q_scr[16 * a:16 * a + 16, :]
                lhs = jnp.concatenate([eye, qb], axis=0)
                o = _dot_t(lhs, _tile(tmp_t, h * NC + b))
                if h in QM:
                    wuk_t[QM.index(h) * NC + b] = _words(o[0:128])
                else:
                    for g in range(16):
                        wuk_f[(QV.index(h) * 16 + g) * NC + b] = o[8 * g:8 * g + 8]
                z[a] = jnp.where(sub == h % 8, o[128:136], z[a])
            z_scr[b] = jnp.concatenate([v * scale for v in z], axis=0)
            return carry

        lax.fori_loop(0, NC, body, 0)
        return [z_scr[b].astype(BF16) for b in range(NC)]

    def scores_first(zs):
        lhs = [jnp.concatenate([eye, zs[b]], axis=0) for b in range(NC)]
        U = 4

        def body(g, carry):
            for i in range(U):
                t = g * U + i
                r0 = pl.multiple_of(t * 128, 128)
                s = None
                for b in range(NC):
                    o = _dot_t(lhs[b], c_v[pl.ds(r0, 128), 128 * b:128 * (b + 1)])
                    c_t[b * NK + t] = _words(o[0:128])
                    s = o[128:160] if s is None else s + o[128:160]
                s_scr[t] = s
            return carry

        lax.fori_loop(0, NK // U, body, 0)

    HALF = NK // 2

    def scores(zs, t0):
        mx = None
        acc = {}

        def tile(t, b):
            o = _dot(zs[b], _tile(c_t, b * NK + t))
            acc[t] = o if b == 0 else acc[t] + o

        groups = [list(range(g0, g0 + 4)) for g0 in range(t0, t0 + HALF, 4)]
        if t0 == 0:
            for b in range(NC - 1):
                for grp in groups[:SLEAD]:
                    for t in grp:
                        tile(t, b)
            for grp in groups[:SLEAD]:
                for t in grp:
                    tile(t, NC - 1)
        for k, grp in enumerate(groups):
            if t0 != 0 or k >= SLEAD:
                for b in range(NC):
                    for t in grp:
                        tile(t, b)
            for t in grp:
                s_scr[t] = acc[t]
                mx = acc[t] if mx is None else jnp.maximum(mx, acc[t])
        return jnp.max(mx, axis=-1, keepdims=True)

    def smax(t0):
        mx = None
        for t in range(t0, t0 + HALF):
            v = s_scr[t]
            mx = v if mx is None else jnp.maximum(mx, v)
        return jnp.max(mx, axis=-1, keepdims=True)

    def softmax_pv(m_a, m_b):
        m = jnp.maximum(m_a, m_b)
        alpha = jnp.exp2(m_a - m)

        def cv(t, b):
            return c_v[128 * t:128 * (t + 1), 128 * b:128 * (b + 1)]

        acc = [None] * NC
        lsum = None
        for t in range(HALF):
            p = jnp.exp2(s_scr[t] - m_a)
            lsum = p if lsum is None else lsum + p
            pb = p.astype(BF16)
            for b in range(NC):
                o = _dot(pb, cv(t, b))
                acc[b] = o if acc[b] is None else acc[b] + o
        lsum = lsum * alpha
        acc = [v * alpha for v in acc]
        for t in range(HALF, HALF + 8):
            p = jnp.exp2(s_scr[t] - m)
            lsum = lsum + p
            pb = p.astype(BF16)
            for b in range(NC):
                acc[b] = acc[b] + _dot(pb, cv(t, b))
        pbs = {}
        for b in range(NC):
            for t in range(HALF + 8, NK):
                if b == 0:
                    p = jnp.exp2(s_scr[t] - m)
                    lsum = lsum + p
                    pbs[t] = p.astype(BF16)
                acc[b] = acc[b] + _dot(pbs[t], cv(t, b))
        linv = 1.0 / jnp.sum(lsum, axis=-1, keepdims=True)
        return acc, linv

    def context(acc, linv):
        for b in range(NC):
            a_scr[:, 128 * b:128 * (b + 1)] = acc[b]
        ctx = [None] * 4

        def mstep(b, h):
            def step():
                a, r = divmod(h, 8)
                o = _dot(row(r, acc[b][8 * a:8 * a + 8]), _tile(wuv_t, VM.index(h) * NC + b))
                ctx[a] = o if ctx[a] is None else ctx[a] + o
            return step

        cur = {}
        done = {}

        def vstep(h, i):
            def step():
                k = VV.index(h)
                if i == 0:
                    xs_ = [bcast_row(a_scr, h, 128 * b) for b in range(NC)]
                    if k >= VLAG:
                        xs_ = [after(done[VV[k - VLAG]], x) for x in xs_]
                    cur["x"] = xs_
                    cur["d"] = 0.0
                p = [cur["x"][b] * wuv_f[(k * 16 + i) * NC + b] for b in range(NC)]
                s = jnp.sum((p[0] + p[1]) + (p[2] + p[3]), axis=-1, keepdims=True)
                cur["d"] = jnp.where(lane == sub + 8 * i, s, cur["d"])
                if i == 0:
                    done[h] = jnp.broadcast_to(s, (8, 128))
                if i == 15:
                    ctxv_scr[k] = _rowsum(cur["d"]) * linv[h:h + 1]
            return step

        _interleave([mstep(b, h) for b in range(NC) for h in VM],
                    [vstep(h, i) for h in VV for i in range(16)])
        for a in range(4):
            if ctx[a] is not None:
                ctx_scr[8 * a:8 * a + 8, :] = ctx[a] * linv[8 * a:8 * a + 8]

    def ctx_row(h):
        return ctxv_scr[VV.index(h)] if h in VV else bcast_row(ctx_scr, h)

    def out_first(i, outs):
        cps["wo", i].wait()
        for h in range(WO_SPLIT[i], WO_SPLIT[i + 1]):
            l = ctx_row(h)
            for j in range(NM):
                t = _dot(l, wo_v[128 * h:128 * (h + 1), 128 * j:128 * (j + 1)])
                outs[j] = t if outs[j] is None else outs[j] + t
        if i < NWO - 1:
            relayout_wo(WO_SPLIT[i], WO_SPLIT[i + 1])

    def relayout_wo(h0, h1):
        nv = len(OV)
        assert OV == tuple(range(nv))

        def body_v(h, carry):
            r0 = pl.multiple_of(h * 128, 128)
            for g in range(16):
                wf = wo_v[pl.ds(r0 + 8 * g, 8), :].astype(F32)
                for j in range(NM):
                    wo_f[(h * 16 + g) * NM + j] = wf[:, 128 * j:128 * (j + 1)]
            return carry

        def body_m(h, carry):
            r0 = pl.multiple_of(h * 128, 128)
            for j in range(NM):
                wo_t[(h - nv) * NM + j] = pltpu.bitcast(wo_v[pl.ds(r0, 128), 128 * j:128 * (j + 1)], I32)
            return carry

        if h0 < min(h1, nv):
            lax.fori_loop(h0, min(h1, nv), body_v, 0)
        if max(h0, nv) < h1:
            lax.fori_loop(max(h0, nv), h1, body_m, 0)

    def out_second():
        outs = [None] * NM
        vacc = [None] * NM

        def mstep(h, j):
            def step():
                t = _dot(ctx_row(h), _tile(wo_t, (h - len(OV)) * NM + j))
                outs[j] = t if outs[j] is None else outs[j] + t
            return step

        part = {}
        groups = [OV[k:k + OG] for k in range(0, len(OV), OG)]

        def o_mac(h, g, m):
            grp = next(x for x in groups if h in x)
            for j in range(NM):
                t = m * wo_f[(OV.index(h) * 16 + g) * NM + j]
                part[j] = t if h == grp[0] else part[j] + t
                if h == grp[-1]:
                    vacc[j] = part[j] if vacc[j] is None else vacc[j] + part[j]
            return part[NM - 1]

        _interleave([mstep(h, j) for j in range(NM) for h in OM], Columns(groups, ctx_row, o_mac, OLAG).steps())
        return [o + _rowsum(v) for o, v in zip(outs, vacc)]

    def ffn_act(xs, mu, rstd, acts, nxt=None):
        acc = {}

        def finish(ft):
            g = rstd * (acc[ft, 0] - mu * csgu_scr[ft])
            u = rstd * (acc[ft, 1] - mu * csgu_scr[NF + ft])
            acts[ft] = g * jax.nn.sigmoid(g) * u

        def mstep(ft, which, j):
            def step():
                o = _dot(xs[j], _tile(gu_t, (which * len(GM) + GM.index(ft)) * NM + j))
                acc[ft, which] = o if j == 0 else acc[ft, which] + o
                if j == NM - 1 and which == 1:
                    finish(ft)
                if nxt is not None and j == 2 and which == 0:
                    for gi, grp in enumerate(nxt.groups[:DEARLY]):
                        if all(acts[x] is not None for x in grp):
                            nxt.start(gi)
            return step

        NTV = len(GV_TILES)
        cur = {}
        vacc = [None] * NTV

        def g_mac(j, g, m):
            for n in range(NTV):
                p = m * gu_f[(j * 16 + g) * NTV + n]
                vacc[n] = p if vacc[n] is None else vacc[n] + p
            return vacc[NTV - 1]

        mx = []
        for f0 in range(0, len(GM), 2):
            for j in range(NM):
                for ft in GM[f0:f0 + 2]:
                    for which in range(2):
                        mx.append(mstep(ft, which, j))
        _interleave(mx, Columns([(j,) for j in range(NM)], lambda j: xs[j], g_mac, GLAG).steps())
        for ft in GV[::-1]:
            if ft < NF - 1:
                acc[ft, 0] = _rowsum(vacc[GV_TILES.index((ft, 0))])
                acc[ft, 1] = _rowsum(vacc[GV_TILES.index((ft, 1))])
                finish(ft)
            else:
                g = rstd * (_rowsum(vacc[GV_TILES.index((ft, 0))]) - mu * csgu_scr[NF + ft])
                acts[ft] = g * jax.nn.sigmoid(g) * pltpu.roll(g, 64, 1)
        return acts

    def down(act, ft, j):
        rows = min(128, F - 128 * ft)
        return _dot(act[:, 0:rows], wd_v[128 * ft:128 * ft + rows, 128 * j:128 * (j + 1)])

    def ffn_residual(xs, mu, rstd, wr):
        xn = [((v - mu) * rstd).astype(BF16).astype(F32) for v in xs]
        rr = None
        for v, w in zip(xn, wr):
            rr = v * w if rr is None else rr + v * w
        sig = jax.nn.sigmoid(jnp.sum(rr, axis=-1, keepdims=True))
        base = [v + n for v, n in zip(xs, xn)]
        zero = [n * 0.0 for n in xn]
        return base, zero, sig

    cps["x"].wait()
    cps["wr"].wait()
    x_all = jnp.broadcast_to(x_v[...].astype(F32), (8, M))
    wr_all = jnp.broadcast_to(wr_v[...].reshape(1, M).astype(F32), (8, M))
    xs = [x_all[:, 128 * j:128 * (j + 1)] for j in range(NM)]
    wr = [wr_all[:, 128 * j:128 * (j + 1)] for j in range(NM)]
    mu, rstd = stats(xs)
    never = jnp.broadcast_to(rstd, (8, 128)) < 0.0

    def after(dep, v):
        return jnp.where(never, dep, v)

    cps["wq"].wait()
    split_wq()
    qacc = [None] * 4
    for j in range(NM):
        q_part(j, xs[j], qacc, True, range(H))
    for a in range(4):
        cs = qacc[a][8:16]
        csq_scr[8 * a:8 * a + 8, :] = cs
        q_scr[16 * a:16 * a + 16, :] = jnp.concatenate([qacc[a][0:8] - mu * cs, zero8], axis=0).astype(BF16)
    cps["wuk"].wait()
    zs = qabs_first(rstd)
    cps["c"].wait()
    scores_first(zs)
    acc, linv = softmax_pv(smax(0), smax(HALF))
    cps["wuv"].wait()
    split_wuv()
    context(acc, linv)
    outs = [None] * NM
    out_first(0, outs)
    cps["wg"].wait()
    transpose_gu(wg_v, 0)
    cps["wu"].wait()
    transpose_gu(wu_v, 1)
    for i in range(1, NWO):
        out_first(i, outs)
    xs = [v + o for v, o in zip(xs, outs)]
    mu, rstd = stats(xs)
    acts = ffn_act(xs, mu, rstd, [None] * NF)
    base, zero, sig = ffn_residual(xs, mu, rstd, wr)
    relayout_wo(WO_SPLIT[-2], WO_SPLIT[-1])
    qacc = [None] * 4
    xs = []

    def down_col(j, fts, y=None):
        for ft in fts:
            o = down(acts[ft], ft, j)
            y = o if y is None else y + o
        return y

    for i in range(NWD - 1):
        if i == NWD - 2:
            acol = {ft: _columns(acts[ft]) for ft in range(D4V)}
        cps["wd", i].wait()
        js = range(WD_SPLIT[i], WD_SPLIT[i + 1])
        for j in js:
            xs.append(base[j] + (zero[j] + down_col(j, range(NF)) * sig))
        for j in js:
            q_part(j, xs[j], qacc, False, range(H) if j < NM - 2 else range(H - QDEFER))
    j = NM - 1
    cps["wd", NWD - 1].wait()
    y = down_col(j, range(D4V, NF))
    q_part(j - 1, xs[j - 1], qacc, False, range(H - QDEFER, H))
    if D4V:
        pv = [None] * D4A
        for ft in range(D4V):
            for g in range(16):
                r0 = 128 * ft + 8 * g
                t = acol[ft][8 * g:8 * g + 8] * wd_v[r0:r0 + 8, 128 * j:128 * (j + 1)].astype(F32)
                k = g % D4A
                pv[k] = t if pv[k] is None else pv[k] + t
        tot = pv[0]
        for v in pv[1:]:
            tot = tot + v
        y = _rowsum(tot) if y is None else y + _rowsum(tot)
    xs.append(base[j] + (zero[j] + y * sig))
    q_part(j, xs[j], qacc, False, range(H))

    mu, rstd = stats(xs)
    qs = [qacc[a] - mu * csq_scr[8 * a:8 * a + 8, :] for a in range(4)]
    zs = qabs(qs, rstd)
    m_a = scores(zs, 0)
    m_b = scores(zs, HALF)
    acc, linv = softmax_pv(m_a, m_b)
    context(acc, linv)
    outs = out_second()
    xs = [v + o for v, o in zip(xs, outs)]
    mu, rstd = stats(xs)
    acts = [None] * NF
    ys = [None] * NM
    yv = [None] * NM
    part = {}
    dgroups = [DV[k:k + DG] for k in range(0, len(DV), DG)]

    def d_mstep(ft, j):
        def step():
            o = down(acts[ft], ft, j)
            ys[j] = o if ys[j] is None else ys[j] + o
        return step

    def d_mac(ft, g, m):
        grp = next(x for x in dgroups if ft in x)
        w = wd_v[128 * ft + 8 * g:128 * ft + 8 * g + 8, :].astype(F32)
        for j in range(NM):
            t = m * w[:, 128 * j:128 * (j + 1)]
            part[j] = t if ft == grp[0] else part[j] + t
            if ft == grp[-1]:
                yv[j] = part[j] if yv[j] is None else yv[j] + part[j]
        return part[NM - 1]

    d_stream = Columns(dgroups, lambda ft: acts[ft], d_mac, DLAG)
    ffn_act(xs, mu, rstd, acts, d_stream)
    base, zero, sig = ffn_residual(xs, mu, rstd, wr)
    dm = [ft for ft in range(NF) if ft not in DV]
    _interleave([d_mstep(ft, j) for ft in dm for j in range(NM)], d_stream.steps())
    if DV:
        ys = [y + _rowsum(v) for y, v in zip(ys, yv)]
    for j in range(NM):
        xo = base[j] + (zero[j] + ys[j] * sig)
        o_ref[:, 128 * j:128 * (j + 1)] = xo[0:1, :].astype(o_ref.dtype)


@jax.jit
def pallas_interleave_layers__compressed_kv_cla__moe_arch_mod__decode_kernel(
        A_x, A_c_kv, A_w_q, A_w_uk, A_w_uv, A_w_o, B_x, B_w_r, B_w_gate, B_w_up, B_w_down):
    del B_x
    any_spec = pl.BlockSpec(memory_space=pl.ANY)

    def tiles(n):
        return pltpu.VMEM((max(n, 1), 64, 128), I32)

    def vregs(n):
        return pltpu.VMEM((max(n, 1), 8, 128), F32)

    out = pl.pallas_call(
        _kernel,
        out_shape=jax.ShapeDtypeStruct((1, M), BF16),
        in_specs=[any_spec] * 10,
        out_specs=pl.BlockSpec(memory_space=pltpu.VMEM),
        scratch_shapes=[
            pltpu.VMEM((1, M), BF16), pltpu.VMEM((M,), BF16),
            pltpu.VMEM((SK, DC), BF16),
            pltpu.VMEM((M * H, D), BF16), pltpu.VMEM((DC * H, D), BF16), pltpu.VMEM((DC * H, D), BF16),
            pltpu.VMEM((H * D, M), BF16),
            pltpu.VMEM((F, M), BF16), pltpu.VMEM((F, M), BF16), pltpu.VMEM((F, M), BF16),
            tiles(H * NM), tiles(H * NC),
            tiles(len(QM) * NC), vregs(len(QV) * 16 * NC),
            tiles(len(VM) * NC), vregs(len(VV) * 16 * NC),
            tiles(len(OM) * NM), vregs(len(OV) * 16 * NM),
            tiles(NC * NK),
            tiles(2 * len(GM) * NM), vregs(len(GV_TILES) * 16 * NM),
            pltpu.VMEM((NK, H, 128), F32), pltpu.VMEM((NC, H, 128), F32), pltpu.VMEM((2 * H, D), BF16),
            pltpu.VMEM((H, DC), F32), pltpu.VMEM((H, D), F32), vregs(len(VV)), pltpu.VMEM((H, D), F32),
            pltpu.VMEM((2 * NF, 8, 128), F32),
            pltpu.SemaphoreType.DMA((8 + NWO + NWD,)),
        ],
        compiler_params=pltpu.CompilerParams(vmem_limit_bytes=110 * 2**20, disable_semaphore_checks=True),
    )(A_x.reshape(1, M), B_w_r, A_c_kv.reshape(SK, DC), A_w_q.reshape(M * H, D),
      A_w_uk.reshape(DC * H, D), A_w_uv.reshape(DC * H, D), A_w_o.reshape(H * D, M),
      B_w_gate.T, B_w_up.T, B_w_down)
    return out.reshape(1, 1, M)
```

```python
import math

import jax
import jax.numpy as jnp
from jax import lax
import jax.experimental.pallas as pl
import jax.experimental.pallas.tpu as pltpu

F32, BF16, I32 = jnp.float32, jnp.bfloat16, jnp.int32
M, H, D, SK, DC, F = 640, 32, 128, 4096, 512, 1728
NM = M // 128
NC = DC // 128
NK = SK // 128
NF = 14
WO_SPLIT = (0, 12, 24, 32)
WD_SPLIT = (0, 2, 4, 5)
NWO = len(WO_SPLIT) - 1
NWD = len(WD_SPLIT) - 1
NN = (((1,), (0,)), ((), ()))
NT = (((1,), (1,)), ((), ()))

QV = tuple(range(12))
VV = tuple(range(11))
OV = tuple(range(12))
GV = tuple(range(9, NF))
DV = tuple(range(4))
D4V = 10
QM = tuple(h for h in range(H) if h not in QV)
VM = tuple(h for h in range(H) if h not in VV)
OM = tuple(h for h in range(H) if h not in OV)
GM = tuple(f for f in range(NF) if f not in GV)
GV_TILES = [(f, w) for f in GV for w in range(2) if (f, w) != (NF - 1, 1)]
QG, OG, DG = 3, 3, 2
QLAG, OLAG, GLAG, DLAG, VLAG = 1, 7, 5, 10, 4
SLEAD, QDEFER, DEARLY, D4A = 2, 8, 2, 4
assert NF - 1 in GV and OV == tuple(range(len(OV)))


def _iota(shape, dim):
    return lax.broadcasted_iota(I32, shape, dim)


def _dot(a, b):
    return lax.dot_general(a, b, NN, preferred_element_type=F32)


def _dot_t(a, b):
    return lax.dot_general(a, b, NT, preferred_element_type=F32)


def _tile(ref, i):
    return pltpu.bitcast(ref[i], BF16)


def _words(v):
    return pltpu.bitcast(v.astype(BF16), I32)


def _interleave(mx, vp):
    nm, nv = len(mx), len(vp)
    iv = 0
    for im, step in enumerate(mx):
        step()
        while iv < (im + 1) * nv // nm:
            vp[iv]()
            iv += 1
    while iv < nv:
        vp[iv]()
        iv += 1


def _rowsum(v):
    return jnp.broadcast_to(jnp.sum(v, axis=0, keepdims=True), v.shape)


def _columns(rowvec):
    return jnp.broadcast_to(rowvec[0:1, :], (128, 128)).T


def _kernel(x_hbm, wr_hbm, c_hbm, wq_hbm, wuk_hbm, wuv_hbm, wo_hbm, wg_hbm, wu_hbm, wd_hbm,
            o_ref,
            x_v, wr_v, c_v, wq_v, wuk_v, wuv_v, wo_v, wg_v, wu_v, wd_v,
            wq_t, tmp_t, wuk_t, wuk_f, wuv_t, wuv_f, wo_t, wo_f, c_t, gu_t, gu_f,
            s_scr, z_scr, q_scr, a_scr, ctx_scr, ctxv_scr, csq_scr, csgu_scr, sems):
    pairs = {"wq": (wq_hbm, wq_v), "x": (x_hbm, x_v), "wr": (wr_hbm, wr_v), "wuk": (wuk_hbm, wuk_v),
             "c": (c_hbm, c_v), "wuv": (wuv_hbm, wuv_v), "wg": (wg_hbm, wg_v), "wu": (wu_hbm, wu_v)}
    for i, (h0, h1) in enumerate(zip(WO_SPLIT[:-1], WO_SPLIT[1:])):
        rows = pl.ds(D * h0, D * (h1 - h0))
        pairs["wo", i] = (wo_hbm.at[rows, :], wo_v.at[rows, :])
    for i, (j0, j1) in enumerate(zip(WD_SPLIT[:-1], WD_SPLIT[1:])):
        cols = pl.ds(128 * j0, 128 * (j1 - j0))
        pairs["wd", i] = (wd_hbm.at[:, cols], wd_v.at[:, cols])
    order = ["wq", "x", "wr", "wuk", "c", "wuv", ("wo", 0), "wg", "wu"]
    order += [("wo", i) for i in range(1, NWO)] + [("wd", i) for i in range(NWD)]
    cps = {k: pltpu.make_async_copy(*pairs[k], sems.at[i]) for i, k in enumerate(order)}
    for k in order:
        cps[k].start()

    sub = _iota((8, 128), 0)
    lane = _iota((8, 128), 1)
    zero8 = jnp.zeros((8, 128), F32)
    eye = (_iota((128, 128), 0) == _iota((128, 128), 1)).astype(BF16)

    def row(r, v):
        return jnp.where(sub == r, v, 0.0)

    def bcast_row(ref, r, c0=0):
        return jnp.broadcast_to(ref[r:r + 1, c0:c0 + 128], (8, 128))

    def split_heads(src_v, nrows, store):
        w32 = src_v.bitcast(I32)

        def transpose8(v):
            for k in (4, 2, 1):
                hi = (sub & k) != 0
                w = list(v)
                for a in range(8):
                    if not a & k:
                        w[a] = jnp.where(hi, pltpu.roll(v[a | k], k, 0), v[a])
                        w[a | k] = jnp.where(hi, v[a | k], pltpu.roll(v[a], 8 - k, 0))
                v = w
            return v

        def body(g, carry):
            base = pl.multiple_of(g * 256, 256)
            blk = lax.shift_right_logical(g, 3)
            rows = pl.ds(pl.multiple_of((g & 7) * 8, 8), 8)
            for hh in range(2):
                ev = transpose8([w32[pl.ds(base + 32 * i + 8 * hh, 8), :] for i in range(8)])
                od = transpose8([w32[pl.ds(base + 32 * i + 16 + 8 * hh, 8), :] for i in range(8)])
                for j in range(8):
                    a, b = ev[j], od[j]
                    h = 16 * hh + 2 * j
                    store(h, blk, (a & 0xFFFF) | (b << 16), rows)
                    store(h + 1, blk, lax.shift_right_logical(a, 16) | (b & -65536), rows)
            return carry

        lax.fori_loop(0, nrows // 16, body, 0)

    def split_wq():
        def store(h, blk, w, rows):
            wq_t[h * NM + blk, rows, :] = w
        split_heads(wq_v, M, store)

    def split_natural(src_v):
        def store(h, blk, w, rows):
            tmp_t[h * NC + blk, rows, :] = w
        split_heads(src_v, DC, store)

    def split_wuv():
        def store(h, blk, w, rows):
            if h in VM:
                wuv_t[VM.index(h) * NC + blk, rows, :] = w
            else:
                tmp_t[VV.index(h) * NC + blk, rows, :] = w
        split_heads(wuv_v, DC, store)

        def body(b, carry):
            for k in range(len(VV)):
                t = _dot_t(eye, _tile(tmp_t, k * NC + b))
                for i in range(16):
                    wuv_f[(k * 16 + i) * NC + b] = t[8 * i:8 * i + 8]
            return carry

        lax.fori_loop(0, NC, body, 0)

    def transpose_gu(src_v, which):
        lhs = jnp.concatenate([eye, jnp.ones((16, 128), BF16)], axis=0)
        fts = list(range(NF - 1)) + ([NF - 1] if which == 1 else [])

        def body(j, carry):
            cols = pl.ds(pl.multiple_of(j * 128, 128), 128)
            css = []
            for k, ft in enumerate(fts):
                if ft < NF - 1:
                    t = src_v[128 * ft:128 * (ft + 1), cols]
                    n = GV_TILES.index((ft, which)) if ft in GV else None
                else:
                    t = jnp.concatenate([wg_v[128 * ft:F, cols], wu_v[128 * ft:F, cols]], axis=0)
                    n = GV_TILES.index((ft, 0))
                o = _dot_t(lhs, t)
                if n is None:
                    gu_t[(which * len(GM) + GM.index(ft)) * NM + j] = _words(o[0:128])
                else:
                    for g in range(16):
                        gu_f[(j * 16 + g) * len(GV_TILES) + n] = o[8 * g:8 * g + 8]
                css.append(carry[k] + o[128:136])
            return tuple(css)

        css = lax.fori_loop(0, NM, body, (zero8,) * len(fts))
        for k, ft in enumerate(fts):
            csgu_scr[which * NF + ft] = css[k]

    class Columns:
        def __init__(self, groups, prep, mac, lag):
            self.groups, self.prep, self.mac, self.lag = groups, prep, mac, lag
            self.cols = {}

        def start(self, i, dep=None):
            if i < len(self.groups) and self.groups[i][0] not in self.cols:
                for key in self.groups[i]:
                    v = self.prep(key)
                    self.cols[key] = _columns(v if dep is None else after(dep, v))

        def steps(self):
            def make(i, g):
                def step():
                    if i == 0 and g == 0:
                        self.start(0)
                        self.start(1)
                    last = None
                    for key in self.groups[i]:
                        last = self.mac(key, g, self.cols[key][8 * g:8 * g + 8])
                    if g == self.lag:
                        self.start(i + 2, last)
                return step

            return [make(i, g) for i in range(len(self.groups)) for g in range(16)]

    def stats(xs):
        tot = xs[0]
        for v in xs[1:]:
            tot = tot + v
        mu = jnp.sum(tot, axis=-1, keepdims=True) * (1.0 / M)
        sq = None
        for v in xs:
            d = v - mu
            sq = d * d if sq is None else sq + d * d
        var = jnp.sum(sq, axis=-1, keepdims=True) * (1.0 / M)
        return mu, lax.rsqrt(var + 1e-5)

    ones_rows = [row(r, 1.0) for r in range(8)]

    def q_part(j, xj, acc, first, heads):
        lhs = []
        for r in range(8):
            l = row(r, xj)
            if first:
                l = jnp.concatenate([l, ones_rows[r]], axis=0)
            lhs.append(l)
        for h in heads:
            if first or h in QM:
                o = _dot(lhs[h % 8], _tile(wq_t, h * NM + j))
                acc[h // 8] = o if acc[h // 8] is None else acc[h // 8] + o
            else:
                o = _dot(xj, _tile(wq_t, h * NM + j))
                acc[4 + h] = o if acc[4 + h] is None else acc[4 + h] + o

    QSCALE = D ** -0.5 * math.log2(math.e)

    def qabs(qs, rstd):
        scale = rstd * QSCALE
        z = [[zero8] * 4 for _ in range(NC)]

        def mstep(b, h):
            def step():
                o = _dot(qs[h // 8], _tile(wuk_t, QM.index(h) * NC + b))
                z[b][h // 8] = jnp.where(sub == h % 8, o, z[b][h // 8])
            return step

        vqacc = {}
        groups = [QV[k:k + QG] for k in range(0, len(QV), QG)]

        def prep_q(h):
            return qs[4 + h]

        def q_mac(h, g, m):
            for b in range(NC):
                p = m * wuk_f[(QV.index(h) * 16 + g) * NC + b]
                vqacc[h, b] = p if g == 0 else vqacc[h, b] + p
                if g == 15:
                    z[b][h // 8] = jnp.where(sub == h % 8, _rowsum(vqacc[h, b]), z[b][h // 8])
            return vqacc[h, NC - 1]

        _interleave([mstep(b, h) for b in range(NC) for h in QM],
                    Columns(groups, prep_q, q_mac, QLAG).steps())
        return [jnp.concatenate([v * scale for v in z[b]], axis=0).astype(BF16) for b in range(NC)]

    def qabs_first(rstd):
        split_natural(wuk_v)
        scale = rstd * QSCALE

        def body(b, carry):
            z = [zero8] * 4
            for h in range(H):
                a = h // 8
                qb = q_scr[16 * a:16 * a + 16, :]
                lhs = jnp.concatenate([eye, qb], axis=0)
                o = _dot_t(lhs, _tile(tmp_t, h * NC + b))
                if h in QM:
                    wuk_t[QM.index(h) * NC + b] = _words(o[0:128])
                else:
                    for g in range(16):
                        wuk_f[(QV.index(h) * 16 + g) * NC + b] = o[8 * g:8 * g + 8]
                z[a] = jnp.where(sub == h % 8, o[128:136], z[a])
            z_scr[b] = jnp.concatenate([v * scale for v in z], axis=0)
            return carry

        lax.fori_loop(0, NC, body, 0)
        return [z_scr[b].astype(BF16) for b in range(NC)]

    def scores_first(zs):
        lhs = [jnp.concatenate([eye, zs[b]], axis=0) for b in range(NC)]
        U = 4

        def body(g, carry):
            for i in range(U):
                t = g * U + i
                r0 = pl.multiple_of(t * 128, 128)
                s = None
                for b in range(NC):
                    o = _dot_t(lhs[b], c_v[pl.ds(r0, 128), 128 * b:128 * (b + 1)])
                    c_t[b * NK + t] = _words(o[0:128])
                    s = o[128:160] if s is None else s + o[128:160]
                s_scr[t] = s
            return carry

        lax.fori_loop(0, NK // U, body, 0)

    HALF = NK // 2

    def scores(zs, t0):
        mx = None
        acc = {}

        def tile(t, b):
            o = _dot(zs[b], _tile(c_t, b * NK + t))
            acc[t] = o if b == 0 else acc[t] + o

        groups = [list(range(g0, g0 + 4)) for g0 in range(t0, t0 + HALF, 4)]
        if t0 == 0:
            for b in range(NC - 1):
                for grp in groups[:SLEAD]:
                    for t in grp:
                        tile(t, b)
            for grp in groups[:SLEAD]:
                for t in grp:
                    tile(t, NC - 1)
        for k, grp in enumerate(groups):
            if t0 != 0 or k >= SLEAD:
                for b in range(NC):
                    for t in grp:
                        tile(t, b)
            for t in grp:
                s_scr[t] = acc[t]
                mx = acc[t] if mx is None else jnp.maximum(mx, acc[t])
        return jnp.max(mx, axis=-1, keepdims=True)

    def smax(t0):
        mx = None
        for t in range(t0, t0 + HALF):
            v = s_scr[t]
            mx = v if mx is None else jnp.maximum(mx, v)
        return jnp.max(mx, axis=-1, keepdims=True)

    def softmax_pv(m_a, m_b):
        m = jnp.maximum(m_a, m_b)
        alpha = jnp.exp2(m_a - m)

        def cv(t, b):
            return c_v[128 * t:128 * (t + 1), 128 * b:128 * (b + 1)]

        acc = [None] * NC
        lsum = None
        for t in range(HALF):
            p = jnp.exp2(s_scr[t] - m_a)
            lsum = p if lsum is None else lsum + p
            pb = p.astype(BF16)
            for b in range(NC):
                o = _dot(pb, cv(t, b))
                acc[b] = o if acc[b] is None else acc[b] + o
        lsum = lsum * alpha
        acc = [v * alpha for v in acc]
        for t in range(HALF, HALF + 8):
            p = jnp.exp2(s_scr[t] - m)
            lsum = lsum + p
            pb = p.astype(BF16)
            for b in range(NC):
                acc[b] = acc[b] + _dot(pb, cv(t, b))
        pbs = {}
        for b in range(NC):
            for t in range(HALF + 8, NK):
                if b == 0:
                    p = jnp.exp2(s_scr[t] - m)
                    lsum = lsum + p
                    pbs[t] = p.astype(BF16)
                acc[b] = acc[b] + _dot(pbs[t], cv(t, b))
        linv = 1.0 / jnp.sum(lsum, axis=-1, keepdims=True)
        return acc, linv

    def context(acc, linv):
        for b in range(NC):
            a_scr[:, 128 * b:128 * (b + 1)] = acc[b]
        ctx = [None] * 4

        def mstep(b, h):
            def step():
                a, r = divmod(h, 8)
                o = _dot(row(r, acc[b][8 * a:8 * a + 8]), _tile(wuv_t, VM.index(h) * NC + b))
                ctx[a] = o if ctx[a] is None else ctx[a] + o
            return step

        cur = {}
        done = {}

        def vstep(h, i):
            def step():
                k = VV.index(h)
                if i == 0:
                    xs_ = [bcast_row(a_scr, h, 128 * b) for b in range(NC)]
                    if k >= VLAG:
                        xs_ = [after(done[VV[k - VLAG]], x) for x in xs_]
                    cur["x"] = xs_
                    cur["d"] = 0.0
                p = [cur["x"][b] * wuv_f[(k * 16 + i) * NC + b] for b in range(NC)]
                s = jnp.sum((p[0] + p[1]) + (p[2] + p[3]), axis=-1, keepdims=True)
                cur["d"] = jnp.where(lane == sub + 8 * i, s, cur["d"])
                if i == 0:
                    done[h] = jnp.broadcast_to(s, (8, 128))
                if i == 15:
                    ctxv_scr[k] = _rowsum(cur["d"]) * linv[h:h + 1]
            return step

        _interleave([mstep(b, h) for b in range(NC) for h in VM],
                    [vstep(h, i) for h in VV for i in range(16)])
        for a in range(4):
            if ctx[a] is not None:
                ctx_scr[8 * a:8 * a + 8, :] = ctx[a] * linv[8 * a:8 * a + 8]

    def ctx_row(h):
        return ctxv_scr[VV.index(h)] if h in VV else bcast_row(ctx_scr, h)

    def out_first(i, outs):
        cps["wo", i].wait()
        for h in range(WO_SPLIT[i], WO_SPLIT[i + 1]):
            l = ctx_row(h)
            for j in range(NM):
                t = _dot(l, wo_v[128 * h:128 * (h + 1), 128 * j:128 * (j + 1)])
                outs[j] = t if outs[j] is None else outs[j] + t
        if i < NWO - 1:
            relayout_wo(WO_SPLIT[i], WO_SPLIT[i + 1])

    def relayout_wo(h0, h1):
        nv = len(OV)
        assert OV == tuple(range(nv))

        def body_v(h, carry):
            r0 = pl.multiple_of(h * 128, 128)
            for g in range(16):
                wf = wo_v[pl.ds(r0 + 8 * g, 8), :].astype(F32)
                for j in range(NM):
                    wo_f[(h * 16 + g) * NM + j] = wf[:, 128 * j:128 * (j + 1)]
            return carry

        def body_m(h, carry):
            r0 = pl.multiple_of(h * 128, 128)
            for j in range(NM):
                wo_t[(h - nv) * NM + j] = pltpu.bitcast(wo_v[pl.ds(r0, 128), 128 * j:128 * (j + 1)], I32)
            return carry

        if h0 < min(h1, nv):
            lax.fori_loop(h0, min(h1, nv), body_v, 0)
        if max(h0, nv) < h1:
            lax.fori_loop(max(h0, nv), h1, body_m, 0)

    def out_second():
        outs = [None] * NM
        vacc = [None] * NM

        def mstep(h, j):
            def step():
                t = _dot(ctx_row(h), _tile(wo_t, (h - len(OV)) * NM + j))
                outs[j] = t if outs[j] is None else outs[j] + t
            return step

        part = {}
        groups = [OV[k:k + OG] for k in range(0, len(OV), OG)]

        def o_mac(h, g, m):
            grp = next(x for x in groups if h in x)
            for j in range(NM):
                t = m * wo_f[(OV.index(h) * 16 + g) * NM + j]
                part[j] = t if h == grp[0] else part[j] + t
                if h == grp[-1]:
                    vacc[j] = part[j] if vacc[j] is None else vacc[j] + part[j]
            return part[NM - 1]

        _interleave([mstep(h, j) for j in range(NM) for h in OM], Columns(groups, ctx_row, o_mac, OLAG).steps())
        return [o + _rowsum(v) for o, v in zip(outs, vacc)]

    def ffn_act(xs, mu, rstd, acts, nxt=None):
        acc = {}

        def finish(ft):
            g = rstd * (acc[ft, 0] - mu * csgu_scr[ft])
            u = rstd * (acc[ft, 1] - mu * csgu_scr[NF + ft])
            acts[ft] = g * jax.nn.sigmoid(g) * u

        def mstep(ft, which, j):
            def step():
                o = _dot(xs[j], _tile(gu_t, (which * len(GM) + GM.index(ft)) * NM + j))
                acc[ft, which] = o if j == 0 else acc[ft, which] + o
                if j == NM - 1 and which == 1:
                    finish(ft)
                if nxt is not None and j == 2 and which == 0:
                    for gi, grp in enumerate(nxt.groups[:DEARLY]):
                        if all(acts[x] is not None for x in grp):
                            nxt.start(gi)
            return step

        NTV = len(GV_TILES)
        cur = {}
        vacc = [None] * NTV

        def g_mac(j, g, m):
            for n in range(NTV):
                p = m * gu_f[(j * 16 + g) * NTV + n]
                vacc[n] = p if vacc[n] is None else vacc[n] + p
            return vacc[NTV - 1]

        mx = []
        for f0 in range(0, len(GM), 2):
            for j in range(NM):
                for ft in GM[f0:f0 + 2]:
                    for which in range(2):
                        mx.append(mstep(ft, which, j))
        _interleave(mx, Columns([(j,) for j in range(NM)], lambda j: xs[j], g_mac, GLAG).steps())
        for ft in GV[::-1]:
            if ft < NF - 1:
                acc[ft, 0] = _rowsum(vacc[GV_TILES.index((ft, 0))])
                acc[ft, 1] = _rowsum(vacc[GV_TILES.index((ft, 1))])
                finish(ft)
            else:
                g = rstd * (_rowsum(vacc[GV_TILES.index((ft, 0))]) - mu * csgu_scr[NF + ft])
                acts[ft] = g * jax.nn.sigmoid(g) * pltpu.roll(g, 64, 1)
        return acts

    def down(act, ft, j):
        rows = min(128, F - 128 * ft)
        return _dot(act[:, 0:rows], wd_v[128 * ft:128 * ft + rows, 128 * j:128 * (j + 1)])

    def ffn_residual(xs, mu, rstd, wr):
        xn = [((v - mu) * rstd).astype(BF16).astype(F32) for v in xs]
        rr = None
        for v, w in zip(xn, wr):
            rr = v * w if rr is None else rr + v * w
        sig = jax.nn.sigmoid(jnp.sum(rr, axis=-1, keepdims=True))
        base = [v + n for v, n in zip(xs, xn)]
        zero = [n * 0.0 for n in xn]
        return base, zero, sig

    cps["x"].wait()
    cps["wr"].wait()
    x_all = jnp.broadcast_to(x_v[...].astype(F32), (8, M))
    wr_all = jnp.broadcast_to(wr_v[...].reshape(1, M).astype(F32), (8, M))
    xs = [x_all[:, 128 * j:128 * (j + 1)] for j in range(NM)]
    wr = [wr_all[:, 128 * j:128 * (j + 1)] for j in range(NM)]
    mu, rstd = stats(xs)
    never = jnp.broadcast_to(rstd, (8, 128)) < 0.0

    def after(dep, v):
        return jnp.where(never, dep, v)

    cps["wq"].wait()
    split_wq()
    qacc = [None] * 4
    for j in range(NM):
        q_part(j, xs[j], qacc, True, range(H))
    for a in range(4):
        cs = qacc[a][8:16]
        csq_scr[8 * a:8 * a + 8, :] = cs
        q_scr[16 * a:16 * a + 16, :] = jnp.concatenate([qacc[a][0:8] - mu * cs, zero8], axis=0).astype(BF16)
    cps["wuk"].wait()
    zs = qabs_first(rstd)
    cps["c"].wait()
    scores_first(zs)
    acc, linv = softmax_pv(smax(0), smax(HALF))
    cps["wuv"].wait()
    split_wuv()
    context(acc, linv)
    outs = [None] * NM
    out_first(0, outs)
    cps["wg"].wait()
    transpose_gu(wg_v, 0)
    cps["wu"].wait()
    transpose_gu(wu_v, 1)
    for i in range(1, NWO):
        out_first(i, outs)
    xs = [v + o for v, o in zip(xs, outs)]
    mu, rstd = stats(xs)
    acts = ffn_act(xs, mu, rstd, [None] * NF)
    base, zero, sig = ffn_residual(xs, mu, rstd, wr)
    relayout_wo(WO_SPLIT[-2], WO_SPLIT[-1])
    qacc = [None] * (4 + H)
    xs = []

    def down_col(j, fts, y=None):
        for ft in fts:
            o = down(acts[ft], ft, j)
            y = o if y is None else y + o
        return y

    for i in range(NWD - 1):
        if i == NWD - 2:
            acol = {ft: _columns(acts[ft]) for ft in range(D4V)}
        cps["wd", i].wait()
        js = range(WD_SPLIT[i], WD_SPLIT[i + 1])
        for j in js:
            xs.append(base[j] + (zero[j] + down_col(j, range(NF)) * sig))
        for j in js:
            q_part(j, xs[j], qacc, False, range(H) if j < NM - 2 else range(H - QDEFER))
    j = NM - 1
    cps["wd", NWD - 1].wait()
    y = down_col(j, range(D4V, NF))
    q_part(j - 1, xs[j - 1], qacc, False, range(H - QDEFER, H))
    if D4V:
        pv = [None] * D4A
        for ft in range(D4V):
            for g in range(16):
                r0 = 128 * ft + 8 * g
                t = acol[ft][8 * g:8 * g + 8] * wd_v[r0:r0 + 8, 128 * j:128 * (j + 1)].astype(F32)
                k = g % D4A
                pv[k] = t if pv[k] is None else pv[k] + t
        tot = pv[0]
        for v in pv[1:]:
            tot = tot + v
        y = _rowsum(tot) if y is None else y + _rowsum(tot)
    xs.append(base[j] + (zero[j] + y * sig))
    q_part(j, xs[j], qacc, False, range(H))

    mu, rstd = stats(xs)
    qs = [None if qacc[a] is None else qacc[a] - mu * csq_scr[8 * a:8 * a + 8, :] for a in range(4)]
    qs += [qacc[4 + h] - mu * bcast_row(csq_scr, h) if h in QV else None for h in range(H)]
    zs = qabs(qs, rstd)
    m_a = scores(zs, 0)
    m_b = scores(zs, HALF)
    acc, linv = softmax_pv(m_a, m_b)
    context(acc, linv)
    outs = out_second()
    xs = [v + o for v, o in zip(xs, outs)]
    mu, rstd = stats(xs)
    acts = [None] * NF
    ys = [None] * NM
    yv = [None] * NM
    part = {}
    dgroups = [DV[k:k + DG] for k in range(0, len(DV), DG)]

    def d_mstep(ft, j):
        def step():
            o = down(acts[ft], ft, j)
            ys[j] = o if ys[j] is None else ys[j] + o
        return step

    def d_mac(ft, g, m):
        grp = next(x for x in dgroups if ft in x)
        w = wd_v[128 * ft + 8 * g:128 * ft + 8 * g + 8, :].astype(F32)
        for j in range(NM):
            t = m * w[:, 128 * j:128 * (j + 1)]
            part[j] = t if ft == grp[0] else part[j] + t
            if ft == grp[-1]:
                yv[j] = part[j] if yv[j] is None else yv[j] + part[j]
        return part[NM - 1]

    d_stream = Columns(dgroups, lambda ft: acts[ft], d_mac, DLAG)
    ffn_act(xs, mu, rstd, acts, d_stream)
    base, zero, sig = ffn_residual(xs, mu, rstd, wr)
    dm = [ft for ft in range(NF) if ft not in DV]
    _interleave([d_mstep(ft, j) for ft in dm for j in range(NM)], d_stream.steps())
    if DV:
        ys = [y + _rowsum(v) for y, v in zip(ys, yv)]
    for j in range(NM):
        xo = base[j] + (zero[j] + ys[j] * sig)
        o_ref[:, 128 * j:128 * (j + 1)] = xo[0:1, :].astype(o_ref.dtype)


@jax.jit
def pallas_interleave_layers__compressed_kv_cla__moe_arch_mod__decode_kernel(
        A_x, A_c_kv, A_w_q, A_w_uk, A_w_uv, A_w_o, B_x, B_w_r, B_w_gate, B_w_up, B_w_down):
    del B_x
    any_spec = pl.BlockSpec(memory_space=pl.ANY)

    def tiles(n):
        return pltpu.VMEM((max(n, 1), 64, 128), I32)

    def vregs(n):
        return pltpu.VMEM((max(n, 1), 8, 128), F32)

    out = pl.pallas_call(
        _kernel,
        out_shape=jax.ShapeDtypeStruct((1, M), BF16),
        in_specs=[any_spec] * 10,
        out_specs=pl.BlockSpec(memory_space=pltpu.VMEM),
        scratch_shapes=[
            pltpu.VMEM((1, M), BF16), pltpu.VMEM((M,), BF16),
            pltpu.VMEM((SK, DC), BF16),
            pltpu.VMEM((M * H, D), BF16), pltpu.VMEM((DC * H, D), BF16), pltpu.VMEM((DC * H, D), BF16),
            pltpu.VMEM((H * D, M), BF16),
            pltpu.VMEM((F, M), BF16), pltpu.VMEM((F, M), BF16), pltpu.VMEM((F, M), BF16),
            tiles(H * NM), tiles(H * NC),
            tiles(len(QM) * NC), vregs(len(QV) * 16 * NC),
            tiles(len(VM) * NC), vregs(len(VV) * 16 * NC),
            tiles(len(OM) * NM), vregs(len(OV) * 16 * NM),
            tiles(NC * NK),
            tiles(2 * len(GM) * NM), vregs(len(GV_TILES) * 16 * NM),
            pltpu.VMEM((NK, H, 128), F32), pltpu.VMEM((NC, H, 128), F32), pltpu.VMEM((2 * H, D), BF16),
            pltpu.VMEM((H, DC), F32), pltpu.VMEM((H, D), F32), vregs(len(VV)), pltpu.VMEM((H, D), F32),
            pltpu.VMEM((2 * NF, 8, 128), F32),
            pltpu.SemaphoreType.DMA((8 + NWO + NWD,)),
        ],
        compiler_params=pltpu.CompilerParams(vmem_limit_bytes=110 * 2**20, disable_semaphore_checks=True),
    )(A_x.reshape(1, M), B_w_r, A_c_kv.reshape(SK, DC), A_w_q.reshape(M * H, D),
      A_w_uk.reshape(DC * H, D), A_w_uv.reshape(DC * H, D), A_w_o.reshape(H * D, M),
      B_w_gate.T, B_w_up.T, B_w_down)
    return out.reshape(1, 1, M)
```

```python
import math

import jax
import jax.numpy as jnp
from jax import lax
import jax.experimental.pallas as pl
import jax.experimental.pallas.tpu as pltpu

F32, BF16, I32 = jnp.float32, jnp.bfloat16, jnp.int32
M, H, D, SK, DC, F = 640, 32, 128, 4096, 512, 1728
NM = M // 128
NC = DC // 128
NK = SK // 128
NF = 14
WO_SPLIT = (0, 12, 24, 32)
WD_SPLIT = (0, 2, 4, 5)
NWO = len(WO_SPLIT) - 1
NWD = len(WD_SPLIT) - 1
NN = (((1,), (0,)), ((), ()))
NT = (((1,), (1,)), ((), ()))

QV = tuple(range(12))
VV = tuple(range(11))
OV = tuple(range(12))
GV = tuple(range(9, NF))
DV = tuple(range(4))
D4V = 10
QM = tuple(h for h in range(H) if h not in QV)
VM = tuple(h for h in range(H) if h not in VV)
OM = tuple(h for h in range(H) if h not in OV)
GM = tuple(f for f in range(NF) if f not in GV)
GV_TILES = [(f, w) for f in GV for w in range(2) if (f, w) != (NF - 1, 1)]
QG, OG, DG = 3, 3, 2
QLAG, OLAG, GLAG, DLAG, VLAG = 1, 7, 5, 10, 4
SLEAD, QDEFER, DEARLY, D4A = 2, 8, 2, 4
assert NF - 1 in GV and OV == tuple(range(len(OV)))


def _iota(shape, dim):
    return lax.broadcasted_iota(I32, shape, dim)


def _dot(a, b):
    return lax.dot_general(a, b, NN, preferred_element_type=F32)


def _dot_t(a, b):
    return lax.dot_general(a, b, NT, preferred_element_type=F32)


def _tile(ref, i):
    return pltpu.bitcast(ref[i], BF16)


def _words(v):
    return pltpu.bitcast(v.astype(BF16), I32)


def _interleave(mx, vp):
    nm, nv = len(mx), len(vp)
    iv = 0
    for im, step in enumerate(mx):
        step()
        while iv < (im + 1) * nv // nm:
            vp[iv]()
            iv += 1
    while iv < nv:
        vp[iv]()
        iv += 1


def _rowsum(v):
    return jnp.broadcast_to(jnp.sum(v, axis=0, keepdims=True), v.shape)


def _columns(rowvec):
    return jnp.broadcast_to(rowvec[0:1, :], (128, 128)).T


def _kernel(x_hbm, wr_hbm, c_hbm, wq_hbm, wuk_hbm, wuv_hbm, wo_hbm, wg_hbm, wu_hbm, wd_hbm,
            o_ref,
            x_v, wr_v, c_v, wq_v, wuk_v, wuv_v, wo_v, wg_v, wu_v, wd_v,
            wq_t, tmp_t, wuk_t, wuk_f, wuv_t, wuv_f, wo_t, wo_f, c_t, gu_t, gu_f,
            s_scr, z_scr, q_scr, a_scr, ctx_scr, ctxv_scr, csq_scr, csgu_scr, sems):
    pairs = {"wq": (wq_hbm, wq_v), "x": (x_hbm, x_v), "wr": (wr_hbm, wr_v), "wuk": (wuk_hbm, wuk_v),
             "c": (c_hbm, c_v), "wuv": (wuv_hbm, wuv_v), "wg": (wg_hbm, wg_v), "wu": (wu_hbm, wu_v)}
    for i, (h0, h1) in enumerate(zip(WO_SPLIT[:-1], WO_SPLIT[1:])):
        rows = pl.ds(D * h0, D * (h1 - h0))
        pairs["wo", i] = (wo_hbm.at[rows, :], wo_v.at[rows, :])
    for i, (j0, j1) in enumerate(zip(WD_SPLIT[:-1], WD_SPLIT[1:])):
        cols = pl.ds(128 * j0, 128 * (j1 - j0))
        pairs["wd", i] = (wd_hbm.at[:, cols], wd_v.at[:, cols])
    order = ["wq", "x", "wr", "wuk", "c", "wuv", ("wo", 0), "wg", "wu"]
    order += [("wo", i) for i in range(1, NWO)] + [("wd", i) for i in range(NWD)]
    cps = {k: pltpu.make_async_copy(*pairs[k], sems.at[i]) for i, k in enumerate(order)}
    for k in order:
        cps[k].start()

    sub = _iota((8, 128), 0)
    lane = _iota((8, 128), 1)
    zero8 = jnp.zeros((8, 128), F32)
    eye = (_iota((128, 128), 0) == _iota((128, 128), 1)).astype(BF16)

    def row(r, v):
        return jnp.where(sub == r, v, 0.0)

    def bcast_row(ref, r, c0=0):
        return jnp.broadcast_to(ref[r:r + 1, c0:c0 + 128], (8, 128))

    def split_heads(src_v, nrows, store):
        def words(row):
            return pltpu.bitcast(src_v[pl.ds(row, 16), :], I32)

        def transpose8(v):
            for k in (4, 2, 1):
                hi = (sub & k) != 0
                w = list(v)
                for a in range(8):
                    if not a & k:
                        w[a] = jnp.where(hi, pltpu.roll(v[a | k], k, 0), v[a])
                        w[a | k] = jnp.where(hi, v[a | k], pltpu.roll(v[a], 8 - k, 0))
                v = w
            return v

        def body(g, carry):
            base = pl.multiple_of(g * 512, 512)
            blk = lax.shift_right_logical(g, 3)
            rows = pl.ds(pl.multiple_of((g & 7) * 8, 8), 8)
            for hh in range(2):
                ev = transpose8([words(base + 64 * i + 16 * hh) for i in range(8)])
                od = transpose8([words(base + 64 * i + 32 + 16 * hh) for i in range(8)])
                for j in range(8):
                    a, b = ev[j], od[j]
                    h = 16 * hh + 2 * j
                    store(h, blk, (a & 0xFFFF) | (b << 16), rows)
                    store(h + 1, blk, lax.shift_right_logical(a, 16) | (b & -65536), rows)
            return carry

        lax.fori_loop(0, nrows // 16, body, 0)

    def split_wq():
        def store(h, blk, w, rows):
            wq_t[h * NM + blk, rows, :] = w
        split_heads(wq_v, M, store)

    def split_natural(src_v):
        def store(h, blk, w, rows):
            tmp_t[h * NC + blk, rows, :] = w
        split_heads(src_v, DC, store)

    def split_wuv():
        def store(h, blk, w, rows):
            if h in VM:
                wuv_t[VM.index(h) * NC + blk, rows, :] = w
            else:
                tmp_t[VV.index(h) * NC + blk, rows, :] = w
        split_heads(wuv_v, DC, store)

        def body(b, carry):
            for k in range(len(VV)):
                t = _dot_t(eye, _tile(tmp_t, k * NC + b))
                for i in range(16):
                    wuv_f[(k * 16 + i) * NC + b] = t[8 * i:8 * i + 8]
            return carry

        lax.fori_loop(0, NC, body, 0)

    def transpose_gu(src_v, which):
        lhs = jnp.concatenate([eye, jnp.ones((16, 128), BF16)], axis=0)
        fts = list(range(NF - 1)) + ([NF - 1] if which == 1 else [])

        def body(j, carry):
            cols = pl.ds(pl.multiple_of(j * 128, 128), 128)
            css = []
            for k, ft in enumerate(fts):
                if ft < NF - 1:
                    t = src_v[128 * ft:128 * (ft + 1), cols]
                    n = GV_TILES.index((ft, which)) if ft in GV else None
                else:
                    t = jnp.concatenate([wg_v[128 * ft:F, cols], wu_v[128 * ft:F, cols]], axis=0)
                    n = GV_TILES.index((ft, 0))
                o = _dot_t(lhs, t)
                if n is None:
                    gu_t[(which * len(GM) + GM.index(ft)) * NM + j] = _words(o[0:128])
                else:
                    for g in range(16):
                        gu_f[(j * 16 + g) * len(GV_TILES) + n] = o[8 * g:8 * g + 8]
                css.append(carry[k] + o[128:136])
            return tuple(css)

        css = lax.fori_loop(0, NM, body, (zero8,) * len(fts))
        for k, ft in enumerate(fts):
            csgu_scr[which * NF + ft] = css[k]

    class Columns:
        def __init__(self, groups, prep, mac, lag):
            self.groups, self.prep, self.mac, self.lag = groups, prep, mac, lag
            self.cols = {}

        def start(self, i, dep=None):
            if i < len(self.groups) and self.groups[i][0] not in self.cols:
                for key in self.groups[i]:
                    v = self.prep(key)
                    self.cols[key] = _columns(v if dep is None else after(dep, v))

        def steps(self):
            def make(i, g):
                def step():
                    if i == 0 and g == 0:
                        self.start(0)
                        self.start(1)
                    last = None
                    for key in self.groups[i]:
                        last = self.mac(key, g, self.cols[key][8 * g:8 * g + 8])
                    if g == self.lag:
                        self.start(i + 2, last)
                return step

            return [make(i, g) for i in range(len(self.groups)) for g in range(16)]

    def stats(xs):
        tot = xs[0]
        for v in xs[1:]:
            tot = tot + v
        mu = jnp.sum(tot, axis=-1, keepdims=True) * (1.0 / M)
        sq = None
        for v in xs:
            d = v - mu
            sq = d * d if sq is None else sq + d * d
        var = jnp.sum(sq, axis=-1, keepdims=True) * (1.0 / M)
        return mu, lax.rsqrt(var + 1e-5)

    ones_rows = [row(r, 1.0) for r in range(8)]

    def q_part(j, xj, acc, first, heads):
        lhs = []
        for r in range(8):
            l = row(r, xj)
            if first:
                l = jnp.concatenate([l, ones_rows[r]], axis=0)
            lhs.append(l)
        for h in heads:
            if first or h in QM:
                o = _dot(lhs[h % 8], _tile(wq_t, h * NM + j))
                acc[h // 8] = o if acc[h // 8] is None else acc[h // 8] + o
            else:
                o = _dot(xj, _tile(wq_t, h * NM + j))
                acc[4 + h] = o if acc[4 + h] is None else acc[4 + h] + o

    QSCALE = D ** -0.5 * math.log2(math.e)

    def qabs(qs, rstd):
        scale = rstd * QSCALE
        z = [[zero8] * 4 for _ in range(NC)]

        def mstep(b, h):
            def step():
                o = _dot(qs[h // 8], _tile(wuk_t, QM.index(h) * NC + b))
                z[b][h // 8] = jnp.where(sub == h % 8, o, z[b][h // 8])
            return step

        vqacc = {}
        groups = [QV[k:k + QG] for k in range(0, len(QV), QG)]

        def prep_q(h):
            return qs[4 + h]

        def q_mac(h, g, m):
            for b in range(NC):
                p = m * wuk_f[(QV.index(h) * 16 + g) * NC + b]
                vqacc[h, b] = p if g == 0 else vqacc[h, b] + p
                if g == 15:
                    z[b][h // 8] = jnp.where(sub == h % 8, _rowsum(vqacc[h, b]), z[b][h // 8])
            return vqacc[h, NC - 1]

        _interleave([mstep(b, h) for b in range(NC) for h in QM],
                    Columns(groups, prep_q, q_mac, QLAG).steps())
        return [jnp.concatenate([v * scale for v in z[b]], axis=0).astype(BF16) for b in range(NC)]

    def qabs_first(rstd):
        split_natural(wuk_v)
        scale = rstd * QSCALE

        def body(b, carry):
            z = [zero8] * 4
            for h in range(H):
                a = h // 8
                qb = q_scr[16 * a:16 * a + 16, :]
                lhs = jnp.concatenate([eye, qb], axis=0)
                o = _dot_t(lhs, _tile(tmp_t, h * NC + b))
                if h in QM:
                    wuk_t[QM.index(h) * NC + b] = _words(o[0:128])
                else:
                    for g in range(16):
                        wuk_f[(QV.index(h) * 16 + g) * NC + b] = o[8 * g:8 * g + 8]
                z[a] = jnp.where(sub == h % 8, o[128:136], z[a])
            z_scr[b] = jnp.concatenate([v * scale for v in z], axis=0)
            return carry

        lax.fori_loop(0, NC, body, 0)
        return [z_scr[b].astype(BF16) for b in range(NC)]

    def scores_first(zs):
        lhs = [jnp.concatenate([eye, zs[b]], axis=0) for b in range(NC)]
        U = 4

        def body(g, carry):
            for i in range(U):
                t = g * U + i
                r0 = pl.multiple_of(t * 128, 128)
                s = None
                for b in range(NC):
                    o = _dot_t(lhs[b], c_v[pl.ds(r0, 128), 128 * b:128 * (b + 1)])
                    c_t[b * NK + t] = _words(o[0:128])
                    s = o[128:160] if s is None else s + o[128:160]
                s_scr[t] = s
            return carry

        lax.fori_loop(0, NK // U, body, 0)

    HALF = NK // 2

    def scores(zs, t0):
        mx = None
        acc = {}

        def tile(t, b):
            o = _dot(zs[b], _tile(c_t, b * NK + t))
            acc[t] = o if b == 0 else acc[t] + o

        groups = [list(range(g0, g0 + 4)) for g0 in range(t0, t0 + HALF, 4)]
        if t0 == 0:
            for b in range(NC - 1):
                for grp in groups[:SLEAD]:
                    for t in grp:
                        tile(t, b)
            for grp in groups[:SLEAD]:
                for t in grp:
                    tile(t, NC - 1)
        for k, grp in enumerate(groups):
            if t0 != 0 or k >= SLEAD:
                for b in range(NC):
                    for t in grp:
                        tile(t, b)
            for t in grp:
                s_scr[t] = acc[t]
                mx = acc[t] if mx is None else jnp.maximum(mx, acc[t])
        return jnp.max(mx, axis=-1, keepdims=True)

    def smax(t0):
        mx = None
        for t in range(t0, t0 + HALF):
            v = s_scr[t]
            mx = v if mx is None else jnp.maximum(mx, v)
        return jnp.max(mx, axis=-1, keepdims=True)

    def softmax_pv(m_a, m_b):
        m = jnp.maximum(m_a, m_b)
        alpha = jnp.exp2(m_a - m)

        def cv(t, b):
            return c_v[128 * t:128 * (t + 1), 128 * b:128 * (b + 1)]

        acc = [None] * NC
        lsum = None
        for t in range(HALF):
            p = jnp.exp2(s_scr[t] - m_a)
            lsum = p if lsum is None else lsum + p
            pb = p.astype(BF16)
            for b in range(NC):
                o = _dot(pb, cv(t, b))
                acc[b] = o if acc[b] is None else acc[b] + o
        lsum = lsum * alpha
        acc = [v * alpha for v in acc]
        for t in range(HALF, HALF + 8):
            p = jnp.exp2(s_scr[t] - m)
            lsum = lsum + p
            pb = p.astype(BF16)
            for b in range(NC):
                acc[b] = acc[b] + _dot(pb, cv(t, b))
        pbs = {}
        for b in range(NC):
            for t in range(HALF + 8, NK):
                if b == 0:
                    p = jnp.exp2(s_scr[t] - m)
                    lsum = lsum + p
                    pbs[t] = p.astype(BF16)
                acc[b] = acc[b] + _dot(pbs[t], cv(t, b))
        linv = 1.0 / jnp.sum(lsum, axis=-1, keepdims=True)
        return acc, linv

    def context(acc, linv):
        for b in range(NC):
            a_scr[:, 128 * b:128 * (b + 1)] = acc[b]
        ctx = [None] * 4

        def mstep(b, h):
            def step():
                a, r = divmod(h, 8)
                o = _dot(row(r, acc[b][8 * a:8 * a + 8]), _tile(wuv_t, VM.index(h) * NC + b))
                ctx[a] = o if ctx[a] is None else ctx[a] + o
            return step

        cur = {}
        done = {}

        def vstep(h, i):
            def step():
                k = VV.index(h)
                if i == 0:
                    xs_ = [bcast_row(a_scr, h, 128 * b) for b in range(NC)]
                    if k >= VLAG:
                        xs_ = [after(done[VV[k - VLAG]], x) for x in xs_]
                    cur["x"] = xs_
                    cur["d"] = 0.0
                p = [cur["x"][b] * wuv_f[(k * 16 + i) * NC + b] for b in range(NC)]
                s = jnp.sum((p[0] + p[1]) + (p[2] + p[3]), axis=-1, keepdims=True)
                cur["d"] = jnp.where(lane == sub + 8 * i, s, cur["d"])
                if i == 0:
                    done[h] = jnp.broadcast_to(s, (8, 128))
                if i == 15:
                    ctxv_scr[k] = _rowsum(cur["d"]) * linv[h:h + 1]
            return step

        _interleave([mstep(b, h) for b in range(NC) for h in VM],
                    [vstep(h, i) for h in VV for i in range(16)])
        for a in range(4):
            if ctx[a] is not None:
                ctx_scr[8 * a:8 * a + 8, :] = ctx[a] * linv[8 * a:8 * a + 8]

    def ctx_row(h):
        return ctxv_scr[VV.index(h)] if h in VV else bcast_row(ctx_scr, h)

    def out_first(i, outs):
        cps["wo", i].wait()
        for h in range(WO_SPLIT[i], WO_SPLIT[i + 1]):
            l = ctx_row(h)
            for j in range(NM):
                t = _dot(l, wo_v[128 * h:128 * (h + 1), 128 * j:128 * (j + 1)])
                outs[j] = t if outs[j] is None else outs[j] + t
        if i < NWO - 1:
            relayout_wo(WO_SPLIT[i], WO_SPLIT[i + 1])

    def relayout_wo(h0, h1):
        nv = len(OV)
        assert OV == tuple(range(nv))

        def body_v(h, carry):
            r0 = pl.multiple_of(h * 128, 128)
            for g in range(16):
                wf = wo_v[pl.ds(r0 + 8 * g, 8), :].astype(F32)
                for j in range(NM):
                    wo_f[(h * 16 + g) * NM + j] = wf[:, 128 * j:128 * (j + 1)]
            return carry

        def body_m(h, carry):
            r0 = pl.multiple_of(h * 128, 128)
            for j in range(NM):
                wo_t[(h - nv) * NM + j] = pltpu.bitcast(wo_v[pl.ds(r0, 128), 128 * j:128 * (j + 1)], I32)
            return carry

        if h0 < min(h1, nv):
            lax.fori_loop(h0, min(h1, nv), body_v, 0)
        if max(h0, nv) < h1:
            lax.fori_loop(max(h0, nv), h1, body_m, 0)

    def out_second():
        outs = [None] * NM
        vacc = [None] * NM

        def mstep(h, j):
            def step():
                t = _dot(ctx_row(h), _tile(wo_t, (h - len(OV)) * NM + j))
                outs[j] = t if outs[j] is None else outs[j] + t
            return step

        part = {}
        groups = [OV[k:k + OG] for k in range(0, len(OV), OG)]

        def o_mac(h, g, m):
            grp = next(x for x in groups if h in x)
            for j in range(NM):
                t = m * wo_f[(OV.index(h) * 16 + g) * NM + j]
                part[j] = t if h == grp[0] else part[j] + t
                if h == grp[-1]:
                    vacc[j] = part[j] if vacc[j] is None else vacc[j] + part[j]
            return part[NM - 1]

        _interleave([mstep(h, j) for j in range(NM) for h in OM], Columns(groups, ctx_row, o_mac, OLAG).steps())
        return [o + _rowsum(v) for o, v in zip(outs, vacc)]

    def ffn_act(xs, mu, rstd, acts, nxt=None):
        acc = {}

        def finish(ft):
            g = rstd * (acc[ft, 0] - mu * csgu_scr[ft])
            u = rstd * (acc[ft, 1] - mu * csgu_scr[NF + ft])
            acts[ft] = g * jax.nn.sigmoid(g) * u

        def mstep(ft, which, j):
            def step():
                o = _dot(xs[j], _tile(gu_t, (which * len(GM) + GM.index(ft)) * NM + j))
                acc[ft, which] = o if j == 0 else acc[ft, which] + o
                if j == NM - 1 and which == 1:
                    finish(ft)
                if nxt is not None and j == 2 and which == 0:
                    for gi, grp in enumerate(nxt.groups[:DEARLY]):
                        if all(acts[x] is not None for x in grp):
                            nxt.start(gi)
            return step

        NTV = len(GV_TILES)
        cur = {}
        vacc = [None] * NTV

        def g_mac(j, g, m):
            for n in range(NTV):
                p = m * gu_f[(j * 16 + g) * NTV + n]
                vacc[n] = p if vacc[n] is None else vacc[n] + p
            return vacc[NTV - 1]

        mx = []
        for f0 in range(0, len(GM), 2):
            for j in range(NM):
                for ft in GM[f0:f0 + 2]:
                    for which in range(2):
                        mx.append(mstep(ft, which, j))
        _interleave(mx, Columns([(j,) for j in range(NM)], lambda j: xs[j], g_mac, GLAG).steps())
        for ft in GV[::-1]:
            if ft < NF - 1:
                acc[ft, 0] = _rowsum(vacc[GV_TILES.index((ft, 0))])
                acc[ft, 1] = _rowsum(vacc[GV_TILES.index((ft, 1))])
                finish(ft)
            else:
                g = rstd * (_rowsum(vacc[GV_TILES.index((ft, 0))]) - mu * csgu_scr[NF + ft])
                acts[ft] = g * jax.nn.sigmoid(g) * pltpu.roll(g, 64, 1)
        return acts

    def down(act, ft, j):
        rows = min(128, F - 128 * ft)
        return _dot(act[:, 0:rows], wd_v[128 * ft:128 * ft + rows, 128 * j:128 * (j + 1)])

    def ffn_residual(xs, mu, rstd, wr):
        xn = [((v - mu) * rstd).astype(BF16).astype(F32) for v in xs]
        rr = None
        for v, w in zip(xn, wr):
            rr = v * w if rr is None else rr + v * w
        sig = jax.nn.sigmoid(jnp.sum(rr, axis=-1, keepdims=True))
        base = [v + n for v, n in zip(xs, xn)]
        zero = [n * 0.0 for n in xn]
        return base, zero, sig

    cps["x"].wait()
    cps["wr"].wait()
    x_all = jnp.broadcast_to(x_v[...].astype(F32), (8, M))
    wr_all = jnp.broadcast_to(wr_v[...].reshape(1, M).astype(F32), (8, M))
    xs = [x_all[:, 128 * j:128 * (j + 1)] for j in range(NM)]
    wr = [wr_all[:, 128 * j:128 * (j + 1)] for j in range(NM)]
    mu, rstd = stats(xs)
    never = jnp.broadcast_to(rstd, (8, 128)) < 0.0

    def after(dep, v):
        return jnp.where(never, dep, v)

    cps["wq"].wait()
    split_wq()
    qacc = [None] * 4
    for j in range(NM):
        q_part(j, xs[j], qacc, True, range(H))
    for a in range(4):
        cs = qacc[a][8:16]
        csq_scr[8 * a:8 * a + 8, :] = cs
        q_scr[16 * a:16 * a + 16, :] = jnp.concatenate([qacc[a][0:8] - mu * cs, zero8], axis=0).astype(BF16)
    cps["wuk"].wait()
    zs = qabs_first(rstd)
    cps["c"].wait()
    scores_first(zs)
    acc, linv = softmax_pv(smax(0), smax(HALF))
    cps["wuv"].wait()
    split_wuv()
    context(acc, linv)
    outs = [None] * NM
    out_first(0, outs)
    cps["wg"].wait()
    transpose_gu(wg_v, 0)
    cps["wu"].wait()
    transpose_gu(wu_v, 1)
    for i in range(1, NWO):
        out_first(i, outs)
    xs = [v + o for v, o in zip(xs, outs)]
    mu, rstd = stats(xs)
    acts = ffn_act(xs, mu, rstd, [None] * NF)
    base, zero, sig = ffn_residual(xs, mu, rstd, wr)
    relayout_wo(WO_SPLIT[-2], WO_SPLIT[-1])
    qacc = [None] * (4 + H)
    xs = []

    def down_col(j, fts, y=None):
        for ft in fts:
            o = down(acts[ft], ft, j)
            y = o if y is None else y + o
        return y

    for i in range(NWD - 1):
        if i == NWD - 2:
            acol = {ft: _columns(acts[ft]) for ft in range(D4V)}
        cps["wd", i].wait()
        js = range(WD_SPLIT[i], WD_SPLIT[i + 1])
        for j in js:
            xs.append(base[j] + (zero[j] + down_col(j, range(NF)) * sig))
        for j in js:
            q_part(j, xs[j], qacc, False, range(H) if j < NM - 2 else range(H - QDEFER))
    j = NM - 1
    cps["wd", NWD - 1].wait()
    y = down_col(j, range(D4V, NF))
    q_part(j - 1, xs[j - 1], qacc, False, range(H - QDEFER, H))
    if D4V:
        pv = [None] * D4A
        for ft in range(D4V):
            for g in range(16):
                r0 = 128 * ft + 8 * g
                t = acol[ft][8 * g:8 * g + 8] * wd_v[r0:r0 + 8, 128 * j:128 * (j + 1)].astype(F32)
                k = g % D4A
                pv[k] = t if pv[k] is None else pv[k] + t
        tot = pv[0]
        for v in pv[1:]:
            tot = tot + v
        y = _rowsum(tot) if y is None else y + _rowsum(tot)
    xs.append(base[j] + (zero[j] + y * sig))
    q_part(j, xs[j], qacc, False, range(H))

    mu, rstd = stats(xs)
    qs = [None if qacc[a] is None else qacc[a] - mu * csq_scr[8 * a:8 * a + 8, :] for a in range(4)]
    qs += [qacc[4 + h] - mu * bcast_row(csq_scr, h) if h in QV else None for h in range(H)]
    zs = qabs(qs, rstd)
    m_a = scores(zs, 0)
    m_b = scores(zs, HALF)
    acc, linv = softmax_pv(m_a, m_b)
    context(acc, linv)
    outs = out_second()
    xs = [v + o for v, o in zip(xs, outs)]
    mu, rstd = stats(xs)
    acts = [None] * NF
    ys = [None] * NM
    yv = [None] * NM
    part = {}
    dgroups = [DV[k:k + DG] for k in range(0, len(DV), DG)]

    def d_mstep(ft, j):
        def step():
            o = down(acts[ft], ft, j)
            ys[j] = o if ys[j] is None else ys[j] + o
        return step

    def d_mac(ft, g, m):
        grp = next(x for x in dgroups if ft in x)
        w = wd_v[128 * ft + 8 * g:128 * ft + 8 * g + 8, :].astype(F32)
        for j in range(NM):
            t = m * w[:, 128 * j:128 * (j + 1)]
            part[j] = t if ft == grp[0] else part[j] + t
            if ft == grp[-1]:
                yv[j] = part[j] if yv[j] is None else yv[j] + part[j]
        return part[NM - 1]

    d_stream = Columns(dgroups, lambda ft: acts[ft], d_mac, DLAG)
    ffn_act(xs, mu, rstd, acts, d_stream)
    base, zero, sig = ffn_residual(xs, mu, rstd, wr)
    dm = [ft for ft in range(NF) if ft not in DV]
    _interleave([d_mstep(ft, j) for ft in dm for j in range(NM)], d_stream.steps())
    if DV:
        ys = [y + _rowsum(v) for y, v in zip(ys, yv)]
    for j in range(NM):
        xo = base[j] + (zero[j] + ys[j] * sig)
        o_ref[:, 128 * j:128 * (j + 1)] = xo[0:1, :].astype(o_ref.dtype)


@jax.jit
def pallas_interleave_layers__compressed_kv_cla__moe_arch_mod__decode_kernel(
        A_x, A_c_kv, A_w_q, A_w_uk, A_w_uv, A_w_o, B_x, B_w_r, B_w_gate, B_w_up, B_w_down):
    del B_x
    any_spec = pl.BlockSpec(memory_space=pl.ANY)

    def tiles(n):
        return pltpu.VMEM((max(n, 1), 64, 128), I32)

    def vregs(n):
        return pltpu.VMEM((max(n, 1), 8, 128), F32)

    out = pl.pallas_call(
        _kernel,
        out_shape=jax.ShapeDtypeStruct((1, M), BF16),
        in_specs=[any_spec] * 10,
        out_specs=pl.BlockSpec(memory_space=pltpu.VMEM),
        scratch_shapes=[
            pltpu.VMEM((1, M), BF16), pltpu.VMEM((M,), BF16),
            pltpu.VMEM((SK, DC), BF16),
            pltpu.VMEM((M * H, D), BF16), pltpu.VMEM((DC * H, D), BF16), pltpu.VMEM((DC * H, D), BF16),
            pltpu.VMEM((H * D, M), BF16),
            pltpu.VMEM((F, M), BF16), pltpu.VMEM((F, M), BF16), pltpu.VMEM((F, M), BF16),
            tiles(H * NM), tiles(H * NC),
            tiles(len(QM) * NC), vregs(len(QV) * 16 * NC),
            tiles(len(VM) * NC), vregs(len(VV) * 16 * NC),
            tiles(len(OM) * NM), vregs(len(OV) * 16 * NM),
            tiles(NC * NK),
            tiles(2 * len(GM) * NM), vregs(len(GV_TILES) * 16 * NM),
            pltpu.VMEM((NK, H, 128), F32), pltpu.VMEM((NC, H, 128), F32), pltpu.VMEM((2 * H, D), BF16),
            pltpu.VMEM((H, DC), F32), pltpu.VMEM((H, D), F32), vregs(len(VV)), pltpu.VMEM((H, D), F32),
            pltpu.VMEM((2 * NF, 8, 128), F32),
            pltpu.SemaphoreType.DMA((8 + NWO + NWD,)),
        ],
        compiler_params=pltpu.CompilerParams(vmem_limit_bytes=110 * 2**20, disable_semaphore_checks=True),
    )(A_x.reshape(1, M), B_w_r, A_c_kv.reshape(SK, DC), A_w_q.reshape(M * H, D),
      A_w_uk.reshape(DC * H, D), A_w_uv.reshape(DC * H, D), A_w_o.reshape(H * D, M),
      B_w_gate.T, B_w_up.T, B_w_down)
    return out.reshape(1, 1, M)
```

```python
import math

import jax
import jax.numpy as jnp
from jax import lax
import jax.experimental.pallas as pl
import jax.experimental.pallas.tpu as pltpu

F32, BF16, I32 = jnp.float32, jnp.bfloat16, jnp.int32
M, H, D, SK, DC, F = 640, 32, 128, 4096, 512, 1728
NM = M // 128
NC = DC // 128
NK = SK // 128
NF = 14
WO_SPLIT = (0, 12, 24, 32)
WD_SPLIT = (0, 2, 4, 5)
WD_CUT = 10
NWO = len(WO_SPLIT) - 1
NWD = len(WD_SPLIT) - 1
NN = (((1,), (0,)), ((), ()))
NT = (((1,), (1,)), ((), ()))

QV = tuple(range(12))
VV = tuple(range(11))
OV = tuple(range(12))
GV = tuple(range(9, NF))
DV = tuple(range(2))
QM = tuple(h for h in range(H) if h not in QV)
VM = tuple(h for h in range(H) if h not in VV)
OM = tuple(h for h in range(H) if h not in OV)
GM = tuple(f for f in range(NF) if f not in GV)
GV_TILES = [(f, w) for f in GV for w in range(2) if (f, w) != (NF - 1, 1)]
QG, OG, DG = 3, 3, 2
QLAG, OLAG, GLAG, DLAG, VLAG = 1, 6, 4, 10, 4
SLEAD, QDEFER, DEARLY, D4A = 2, 4, 1, 4
assert NF - 1 in GV and OV == tuple(range(len(OV)))


def _iota(shape, dim):
    return lax.broadcasted_iota(I32, shape, dim)


def _dot(a, b):
    return lax.dot_general(a, b, NN, preferred_element_type=F32)


def _dot_t(a, b):
    return lax.dot_general(a, b, NT, preferred_element_type=F32)


def _tile(ref, i):
    return pltpu.bitcast(ref[i], BF16)


def _words(v):
    return pltpu.bitcast(v.astype(BF16), I32)


def _interleave(mx, vp):
    nm, nv = len(mx), len(vp)
    iv = 0
    for im, step in enumerate(mx):
        step()
        while iv < (im + 1) * nv // nm:
            vp[iv]()
            iv += 1
    while iv < nv:
        vp[iv]()
        iv += 1


def _rowsum(v):
    return jnp.broadcast_to(jnp.sum(v, axis=0, keepdims=True), v.shape)


def _columns(rowvec):
    return jnp.broadcast_to(rowvec[0:1, :], (128, 128)).T


def _kernel(x_hbm, wr_hbm, c_hbm, wq_hbm, wuk_hbm, wuv_hbm, wo_hbm, wg_hbm, wu_hbm, wd_hbm,
            o_ref,
            x_v, wr_v, c_v, wq_v, wuk_v, wuv_v, wo_v, wg_v, wu_v, wd_v,
            wq_t, tmp_t, wuk_t, wuk_f, wuv_t, wuv_f, wo_t, wo_f, c_t, gu_t, gu_f,
            s_scr, z_scr, q_scr, a_scr, ctx_scr, ctxv_scr, csq_scr, csgu_scr, sems):
    pairs = {"wq": (wq_hbm, wq_v), "x": (x_hbm, x_v), "wr": (wr_hbm, wr_v), "wuk": (wuk_hbm, wuk_v),
             "c": (c_hbm, c_v), "wuv": (wuv_hbm, wuv_v), "wg": (wg_hbm, wg_v), "wu": (wu_hbm, wu_v)}
    for i, (h0, h1) in enumerate(zip(WO_SPLIT[:-1], WO_SPLIT[1:])):
        rows = pl.ds(D * h0, D * (h1 - h0))
        pairs["wo", i] = (wo_hbm.at[rows, :], wo_v.at[rows, :])
    for i, (j0, j1) in enumerate(zip(WD_SPLIT[:-1], WD_SPLIT[1:])):
        cols = pl.ds(128 * j0, 128 * (j1 - j0))
        pairs["wd", i] = (wd_hbm.at[:, cols], wd_v.at[:, cols])
    last_cols = pl.ds(M - 128, 128)
    pairs["wd", NWD - 1] = (wd_hbm.at[pl.ds(0, 128 * WD_CUT), last_cols], wd_v.at[pl.ds(0, 128 * WD_CUT), last_cols])
    pairs["wd", NWD] = (wd_hbm.at[pl.ds(128 * WD_CUT, F - 128 * WD_CUT), last_cols],
                        wd_v.at[pl.ds(128 * WD_CUT, F - 128 * WD_CUT), last_cols])
    order = ["wq", "x", "wr", "wuk", "c", "wuv", ("wo", 0), "wg", "wu"]
    order += [("wo", i) for i in range(1, NWO)] + [("wd", i) for i in range(NWD + 1)]
    cps = {k: pltpu.make_async_copy(*pairs[k], sems.at[i]) for i, k in enumerate(order)}
    for k in order:
        cps[k].start()

    sub = _iota((8, 128), 0)
    lane = _iota((8, 128), 1)
    zero8 = jnp.zeros((8, 128), F32)
    eye = (_iota((128, 128), 0) == _iota((128, 128), 1)).astype(BF16)

    def row(r, v):
        return jnp.where(sub == r, v, 0.0)

    def bcast_row(ref, r, c0=0):
        return jnp.broadcast_to(ref[r:r + 1, c0:c0 + 128], (8, 128))

    def split_heads(src_v, nrows, store):
        def words(row):
            return pltpu.bitcast(src_v[pl.ds(row, 16), :], I32)

        def transpose8(v):
            for k in (4, 2, 1):
                hi = (sub & k) != 0
                w = list(v)
                for a in range(8):
                    if not a & k:
                        w[a] = jnp.where(hi, pltpu.roll(v[a | k], k, 0), v[a])
                        w[a | k] = jnp.where(hi, v[a | k], pltpu.roll(v[a], 8 - k, 0))
                v = w
            return v

        def body(g, carry):
            base = pl.multiple_of(g * 512, 512)
            blk = lax.shift_right_logical(g, 3)
            rows = pl.ds(pl.multiple_of((g & 7) * 8, 8), 8)
            for hh in range(2):
                ev = transpose8([words(base + 64 * i + 16 * hh) for i in range(8)])
                od = transpose8([words(base + 64 * i + 32 + 16 * hh) for i in range(8)])
                for j in range(8):
                    a, b = ev[j], od[j]
                    h = 16 * hh + 2 * j
                    store(h, blk, (a & 0xFFFF) | (b << 16), rows)
                    store(h + 1, blk, lax.shift_right_logical(a, 16) | (b & -65536), rows)
            return carry

        lax.fori_loop(0, nrows // 16, body, 0)

    def split_wq():
        def store(h, blk, w, rows):
            wq_t[h * NM + blk, rows, :] = w
        split_heads(wq_v, M, store)

    def split_natural(src_v):
        def store(h, blk, w, rows):
            tmp_t[h * NC + blk, rows, :] = w
        split_heads(src_v, DC, store)

    def split_wuv():
        def store(h, blk, w, rows):
            if h in VM:
                wuv_t[VM.index(h) * NC + blk, rows, :] = w
            else:
                tmp_t[VV.index(h) * NC + blk, rows, :] = w
        split_heads(wuv_v, DC, store)

        def body(b, carry):
            for k in range(len(VV)):
                t = _dot_t(eye, _tile(tmp_t, k * NC + b))
                for i in range(16):
                    wuv_f[(k * 16 + i) * NC + b] = t[8 * i:8 * i + 8]
            return carry

        lax.fori_loop(0, NC, body, 0)

    def transpose_gu(src_v, which):
        lhs = jnp.concatenate([eye, jnp.ones((16, 128), BF16)], axis=0)
        fts = list(range(NF - 1)) + ([NF - 1] if which == 1 else [])

        def body(j, carry):
            cols = pl.ds(pl.multiple_of(j * 128, 128), 128)
            css = []
            for k, ft in enumerate(fts):
                if ft < NF - 1:
                    t = src_v[128 * ft:128 * (ft + 1), cols]
                    n = GV_TILES.index((ft, which)) if ft in GV else None
                else:
                    t = jnp.concatenate([wg_v[128 * ft:F, cols], wu_v[128 * ft:F, cols]], axis=0)
                    n = GV_TILES.index((ft, 0))
                o = _dot_t(lhs, t)
                if n is None:
                    gu_t[(which * len(GM) + GM.index(ft)) * NM + j] = _words(o[0:128])
                else:
                    for g in range(16):
                        gu_f[(j * 16 + g) * len(GV_TILES) + n] = o[8 * g:8 * g + 8]
                css.append(carry[k] + o[128:136])
            return tuple(css)

        css = lax.fori_loop(0, NM, body, (zero8,) * len(fts))
        for k, ft in enumerate(fts):
            csgu_scr[which * NF + ft] = css[k]

    class Columns:
        def __init__(self, groups, prep, mac, lag):
            self.groups, self.prep, self.mac, self.lag = groups, prep, mac, lag
            self.cols = {}

        def start(self, i, dep=None):
            if i < len(self.groups) and self.groups[i][0] not in self.cols:
                for key in self.groups[i]:
                    v = self.prep(key)
                    self.cols[key] = _columns(v if dep is None else after(dep, v))

        def steps(self):
            def make(i, g):
                def step():
                    if i == 0 and g == 0:
                        self.start(0)
                        self.start(1)
                    last = None
                    for key in self.groups[i]:
                        last = self.mac(key, g, self.cols[key][8 * g:8 * g + 8])
                    if g == self.lag:
                        self.start(i + 2, last)
                return step

            return [make(i, g) for i in range(len(self.groups)) for g in range(16)]

    def stats(xs):
        tot = xs[0]
        for v in xs[1:]:
            tot = tot + v
        mu = jnp.sum(tot, axis=-1, keepdims=True) * (1.0 / M)
        sq = None
        for v in xs:
            d = v - mu
            sq = d * d if sq is None else sq + d * d
        var = jnp.sum(sq, axis=-1, keepdims=True) * (1.0 / M)
        return mu, lax.rsqrt(var + 1e-5)

    ones_rows = [row(r, 1.0) for r in range(8)]

    def q_part(j, xj, acc, first, heads):
        lhs = []
        for r in range(8):
            l = row(r, xj)
            if first:
                l = jnp.concatenate([l, ones_rows[r]], axis=0)
            lhs.append(l)
        for h in heads:
            if first or h in QM:
                o = _dot(lhs[h % 8], _tile(wq_t, h * NM + j))
                acc[h // 8] = o if acc[h // 8] is None else acc[h // 8] + o
            else:
                o = _dot(xj, _tile(wq_t, h * NM + j))
                acc[4 + h] = o if acc[4 + h] is None else acc[4 + h] + o

    QSCALE = D ** -0.5 * math.log2(math.e)

    def qabs(qs, rstd):
        scale = rstd * QSCALE
        z = [[zero8] * 4 for _ in range(NC)]

        def mstep(b, h):
            def step():
                o = _dot(qs[h // 8], _tile(wuk_t, QM.index(h) * NC + b))
                z[b][h // 8] = jnp.where(sub == h % 8, o, z[b][h // 8])
            return step

        vqacc = {}
        groups = [QV[k:k + QG] for k in range(0, len(QV), QG)]

        def prep_q(h):
            return qs[4 + h]

        def q_mac(h, g, m):
            for b in range(NC):
                p = m * wuk_f[(QV.index(h) * 16 + g) * NC + b]
                vqacc[h, b] = p if g == 0 else vqacc[h, b] + p
                if g == 15:
                    z[b][h // 8] = jnp.where(sub == h % 8, _rowsum(vqacc[h, b]), z[b][h // 8])
            return vqacc[h, NC - 1]

        _interleave([mstep(b, h) for b in range(NC) for h in QM],
                    Columns(groups, prep_q, q_mac, QLAG).steps())
        return [jnp.concatenate([v * scale for v in z[b]], axis=0).astype(BF16) for b in range(NC)]

    def qabs_first(rstd):
        split_natural(wuk_v)
        scale = rstd * QSCALE

        def body(b, carry):
            z = [zero8] * 4
            for h in range(H):
                a = h // 8
                qb = q_scr[16 * a:16 * a + 16, :]
                lhs = jnp.concatenate([eye, qb], axis=0)
                o = _dot_t(lhs, _tile(tmp_t, h * NC + b))
                if h in QM:
                    wuk_t[QM.index(h) * NC + b] = _words(o[0:128])
                else:
                    for g in range(16):
                        wuk_f[(QV.index(h) * 16 + g) * NC + b] = o[8 * g:8 * g + 8]
                z[a] = jnp.where(sub == h % 8, o[128:136], z[a])
            z_scr[b] = jnp.concatenate([v * scale for v in z], axis=0)
            return carry

        lax.fori_loop(0, NC, body, 0)
        return [z_scr[b].astype(BF16) for b in range(NC)]

    def scores_first(zs):
        lhs = [jnp.concatenate([eye, zs[b]], axis=0) for b in range(NC)]
        U = 4

        def body(g, carry):
            for i in range(U):
                t = g * U + i
                r0 = pl.multiple_of(t * 128, 128)
                s = None
                for b in range(NC):
                    o = _dot_t(lhs[b], c_v[pl.ds(r0, 128), 128 * b:128 * (b + 1)])
                    c_t[b * NK + t] = _words(o[0:128])
                    s = o[128:160] if s is None else s + o[128:160]
                s_scr[t] = s
            return carry

        lax.fori_loop(0, NK // U, body, 0)

    HALF = NK // 2

    def scores(zs, t0):
        mx = None
        acc = {}

        def tile(t, b):
            o = _dot(zs[b], _tile(c_t, b * NK + t))
            acc[t] = o if b == 0 else acc[t] + o

        groups = [list(range(g0, g0 + 4)) for g0 in range(t0, t0 + HALF, 4)]
        if t0 == 0:
            for b in range(NC - 1):
                for grp in groups[:SLEAD]:
                    for t in grp:
                        tile(t, b)
            for grp in groups[:SLEAD]:
                for t in grp:
                    tile(t, NC - 1)
        for k, grp in enumerate(groups):
            if t0 != 0 or k >= SLEAD:
                for b in range(NC):
                    for t in grp:
                        tile(t, b)
            for t in grp:
                s_scr[t] = acc[t]
                mx = acc[t] if mx is None else jnp.maximum(mx, acc[t])
        return jnp.max(mx, axis=-1, keepdims=True)

    def smax(t0):
        mx = None
        for t in range(t0, t0 + HALF):
            v = s_scr[t]
            mx = v if mx is None else jnp.maximum(mx, v)
        return jnp.max(mx, axis=-1, keepdims=True)

    def softmax_pv(m_a, m_b):
        m = jnp.maximum(m_a, m_b)
        alpha = jnp.exp2(m_a - m)

        def cv(t, b):
            return c_v[128 * t:128 * (t + 1), 128 * b:128 * (b + 1)]

        acc = [None] * NC
        lsum = None
        for t in range(HALF):
            p = jnp.exp2(s_scr[t] - m_a)
            lsum = p if lsum is None else lsum + p
            pb = p.astype(BF16)
            for b in range(NC):
                o = _dot(pb, cv(t, b))
                acc[b] = o if acc[b] is None else acc[b] + o
        lsum = lsum * alpha
        acc = [v * alpha for v in acc]
        for t in range(HALF, HALF + 8):
            p = jnp.exp2(s_scr[t] - m)
            lsum = lsum + p
            pb = p.astype(BF16)
            for b in range(NC):
                acc[b] = acc[b] + _dot(pb, cv(t, b))
        pbs = {}
        for b in range(NC):
            for t in range(HALF + 8, NK):
                if b == 0:
                    p = jnp.exp2(s_scr[t] - m)
                    lsum = lsum + p
                    pbs[t] = p.astype(BF16)
                acc[b] = acc[b] + _dot(pbs[t], cv(t, b))
        linv = 1.0 / jnp.sum(lsum, axis=-1, keepdims=True)
        return acc, linv

    def context(acc, linv):
        for b in range(NC):
            a_scr[:, 128 * b:128 * (b + 1)] = acc[b]
        ctx = [None] * 4

        def mstep(b, h):
            def step():
                a, r = divmod(h, 8)
                o = _dot(row(r, acc[b][8 * a:8 * a + 8]), _tile(wuv_t, VM.index(h) * NC + b))
                ctx[a] = o if ctx[a] is None else ctx[a] + o
            return step

        cur = {}
        done = {}

        def vstep(h, i):
            def step():
                k = VV.index(h)
                if i == 0:
                    xs_ = [bcast_row(a_scr, h, 128 * b) for b in range(NC)]
                    if k >= VLAG:
                        xs_ = [after(done[VV[k - VLAG]], x) for x in xs_]
                    cur["x"] = xs_
                    cur["d"] = 0.0
                p = [cur["x"][b] * wuv_f[(k * 16 + i) * NC + b] for b in range(NC)]
                s = jnp.sum((p[0] + p[1]) + (p[2] + p[3]), axis=-1, keepdims=True)
                cur["d"] = jnp.where(lane == sub + 8 * i, s, cur["d"])
                if i == 0:
                    done[h] = jnp.broadcast_to(s, (8, 128))
                if i == 15:
                    ctxv_scr[k] = _rowsum(cur["d"]) * linv[h:h + 1]
            return step

        _interleave([mstep(b, h) for b in range(NC) for h in VM],
                    [vstep(h, i) for h in VV for i in range(16)])
        for a in range(4):
            if ctx[a] is not None:
                ctx_scr[8 * a:8 * a + 8, :] = ctx[a] * linv[8 * a:8 * a + 8]

    def ctx_row(h):
        return ctxv_scr[VV.index(h)] if h in VV else bcast_row(ctx_scr, h)

    def out_first(i, outs):
        cps["wo", i].wait()
        for h in range(WO_SPLIT[i], WO_SPLIT[i + 1]):
            l = ctx_row(h)
            for j in range(NM):
                t = _dot(l, wo_v[128 * h:128 * (h + 1), 128 * j:128 * (j + 1)])
                outs[j] = t if outs[j] is None else outs[j] + t
        if i < NWO - 1:
            relayout_wo(WO_SPLIT[i], WO_SPLIT[i + 1])

    def relayout_wo(h0, h1):
        nv = len(OV)
        assert OV == tuple(range(nv))

        def body_v(h, carry):
            r0 = pl.multiple_of(h * 128, 128)
            for g in range(16):
                wf = wo_v[pl.ds(r0 + 8 * g, 8), :].astype(F32)
                for j in range(NM):
                    wo_f[(h * 16 + g) * NM + j] = wf[:, 128 * j:128 * (j + 1)]
            return carry

        def body_m(h, carry):
            r0 = pl.multiple_of(h * 128, 128)
            for j in range(NM):
                wo_t[(h - nv) * NM + j] = pltpu.bitcast(wo_v[pl.ds(r0, 128), 128 * j:128 * (j + 1)], I32)
            return carry

        if h0 < min(h1, nv):
            lax.fori_loop(h0, min(h1, nv), body_v, 0)
        if max(h0, nv) < h1:
            lax.fori_loop(max(h0, nv), h1, body_m, 0)

    def out_second():
        outs = [None] * NM
        vacc = [None] * NM

        def mstep(h, j):
            def step():
                t = _dot(ctx_row(h), _tile(wo_t, (h - len(OV)) * NM + j))
                outs[j] = t if outs[j] is None else outs[j] + t
            return step

        part = {}
        groups = [OV[k:k + OG] for k in range(0, len(OV), OG)]

        def o_mac(h, g, m):
            grp = next(x for x in groups if h in x)
            for j in range(NM):
                t = m * wo_f[(OV.index(h) * 16 + g) * NM + j]
                part[j] = t if h == grp[0] else part[j] + t
                if h == grp[-1]:
                    vacc[j] = part[j] if vacc[j] is None else vacc[j] + part[j]
            return part[NM - 1]

        _interleave([mstep(h, j) for j in range(NM) for h in OM], Columns(groups, ctx_row, o_mac, OLAG).steps())
        return [o + _rowsum(v) for o, v in zip(outs, vacc)]

    def ffn_act(xs, mu, rstd, acts, nxt=None):
        acc = {}

        def finish(ft):
            g = rstd * (acc[ft, 0] - mu * csgu_scr[ft])
            u = rstd * (acc[ft, 1] - mu * csgu_scr[NF + ft])
            acts[ft] = g * jax.nn.sigmoid(g) * u

        def mstep(ft, which, j):
            def step():
                o = _dot(xs[j], _tile(gu_t, (which * len(GM) + GM.index(ft)) * NM + j))
                acc[ft, which] = o if j == 0 else acc[ft, which] + o
                if j == NM - 1 and which == 1:
                    finish(ft)
                if nxt is not None and j == 2 and which == 0:
                    for gi, grp in enumerate(nxt.groups[:DEARLY]):
                        if all(acts[x] is not None for x in grp):
                            nxt.start(gi)
            return step

        NTV = len(GV_TILES)
        cur = {}
        vacc = [None] * NTV

        def g_mac(j, g, m):
            for n in range(NTV):
                p = m * gu_f[(j * 16 + g) * NTV + n]
                vacc[n] = p if vacc[n] is None else vacc[n] + p
            return vacc[NTV - 1]

        mx = []
        for f0 in range(0, len(GM), 2):
            for j in range(NM):
                for ft in GM[f0:f0 + 2]:
                    for which in range(2):
                        mx.append(mstep(ft, which, j))
        _interleave(mx, Columns([(j,) for j in range(NM)], lambda j: xs[j], g_mac, GLAG).steps())
        for ft in GV[::-1]:
            if ft < NF - 1:
                acc[ft, 0] = _rowsum(vacc[GV_TILES.index((ft, 0))])
                acc[ft, 1] = _rowsum(vacc[GV_TILES.index((ft, 1))])
                finish(ft)
            else:
                g = rstd * (_rowsum(vacc[GV_TILES.index((ft, 0))]) - mu * csgu_scr[NF + ft])
                acts[ft] = g * jax.nn.sigmoid(g) * pltpu.roll(g, 64, 1)
        return acts

    def down(act, ft, j):
        rows = min(128, F - 128 * ft)
        return _dot(act[:, 0:rows], wd_v[128 * ft:128 * ft + rows, 128 * j:128 * (j + 1)])

    def ffn_residual(xs, mu, rstd, wr):
        xn = [((v - mu) * rstd).astype(BF16).astype(F32) for v in xs]
        rr = None
        for v, w in zip(xn, wr):
            rr = v * w if rr is None else rr + v * w
        sig = jax.nn.sigmoid(jnp.sum(rr, axis=-1, keepdims=True))
        base = [v + n for v, n in zip(xs, xn)]
        zero = [n * 0.0 for n in xn]
        return base, zero, sig

    cps["x"].wait()
    cps["wr"].wait()
    x_all = jnp.broadcast_to(x_v[...].astype(F32), (8, M))
    wr_all = jnp.broadcast_to(wr_v[...].reshape(1, M).astype(F32), (8, M))
    xs = [x_all[:, 128 * j:128 * (j + 1)] for j in range(NM)]
    wr = [wr_all[:, 128 * j:128 * (j + 1)] for j in range(NM)]
    mu, rstd = stats(xs)
    never = jnp.broadcast_to(rstd, (8, 128)) < 0.0

    def after(dep, v):
        return jnp.where(never, dep, v)

    cps["wq"].wait()
    split_wq()
    qacc = [None] * 4
    for j in range(NM):
        q_part(j, xs[j], qacc, True, range(H))
    for a in range(4):
        cs = qacc[a][8:16]
        csq_scr[8 * a:8 * a + 8, :] = cs
        q_scr[16 * a:16 * a + 16, :] = jnp.concatenate([qacc[a][0:8] - mu * cs, zero8], axis=0).astype(BF16)
    cps["wuk"].wait()
    zs = qabs_first(rstd)
    cps["c"].wait()
    scores_first(zs)
    acc, linv = softmax_pv(smax(0), smax(HALF))
    cps["wuv"].wait()
    split_wuv()
    context(acc, linv)
    outs = [None] * NM
    out_first(0, outs)
    cps["wg"].wait()
    transpose_gu(wg_v, 0)
    cps["wu"].wait()
    transpose_gu(wu_v, 1)
    for i in range(1, NWO):
        out_first(i, outs)
    xs = [v + o for v, o in zip(xs, outs)]
    mu, rstd = stats(xs)
    acts = ffn_act(xs, mu, rstd, [None] * NF)
    base, zero, sig = ffn_residual(xs, mu, rstd, wr)
    relayout_wo(WO_SPLIT[-2], WO_SPLIT[-1])
    qacc = [None] * (4 + H)
    xs = []

    def down_col(j, fts, y=None):
        for ft in fts:
            o = down(acts[ft], ft, j)
            y = o if y is None else y + o
        return y

    for i in range(NWD - 1):
        if i == NWD - 2:
            acol = {ft: _columns(acts[ft]) for ft in range(NF)}
        cps["wd", i].wait()
        js = range(WD_SPLIT[i], WD_SPLIT[i + 1])
        for j in js:
            xs.append(base[j] + (zero[j] + down_col(j, range(NF)) * sig))
        for j in js:
            q_part(j, xs[j], qacc, False, range(H) if j < NM - 2 else range(H - QDEFER))
    j = NM - 1
    cps["wd", NWD - 1].wait()
    pv = [None] * D4A

    def down_vpu(fts):
        for ft in fts:
            for g in range(min(16, (F - 128 * ft) // 8)):
                r0 = 128 * ft + 8 * g
                t = acol[ft][8 * g:8 * g + 8] * wd_v[r0:r0 + 8, 128 * j:128 * (j + 1)].astype(F32)
                k = g % D4A
                pv[k] = t if pv[k] is None else pv[k] + t

    down_vpu(range(WD_CUT))
    cps["wd", NWD].wait()
    q_part(j - 1, xs[j - 1], qacc, False, range(H - QDEFER, H))
    down_vpu(range(WD_CUT, NF))
    tot = pv[0]
    for v in pv[1:]:
        tot = tot + v
    y = _rowsum(tot)
    xs.append(base[j] + (zero[j] + y * sig))
    q_part(j, xs[j], qacc, False, range(H))

    mu, rstd = stats(xs)
    qs = [None if qacc[a] is None else qacc[a] - mu * csq_scr[8 * a:8 * a + 8, :] for a in range(4)]
    qs += [qacc[4 + h] - mu * bcast_row(csq_scr, h) if h in QV else None for h in range(H)]
    zs = qabs(qs, rstd)
    m_a = scores(zs, 0)
    m_b = scores(zs, HALF)
    acc, linv = softmax_pv(m_a, m_b)
    context(acc, linv)
    outs = out_second()
    xs = [v + o for v, o in zip(xs, outs)]
    mu, rstd = stats(xs)
    acts = [None] * NF
    ys = [None] * NM
    yv = [None] * NM
    part = {}
    dgroups = [DV[k:k + DG] for k in range(0, len(DV), DG)]

    def d_mstep(ft, j):
        def step():
            o = down(acts[ft], ft, j)
            ys[j] = o if ys[j] is None else ys[j] + o
        return step

    def d_mac(ft, g, m):
        grp = next(x for x in dgroups if ft in x)
        w = wd_v[128 * ft + 8 * g:128 * ft + 8 * g + 8, :].astype(F32)
        for j in range(NM):
            t = m * w[:, 128 * j:128 * (j + 1)]
            part[j] = t if ft == grp[0] else part[j] + t
            if ft == grp[-1]:
                yv[j] = part[j] if yv[j] is None else yv[j] + part[j]
        return part[NM - 1]

    d_stream = Columns(dgroups, lambda ft: acts[ft], d_mac, DLAG)
    ffn_act(xs, mu, rstd, acts, d_stream)
    base, zero, sig = ffn_residual(xs, mu, rstd, wr)
    dm = [ft for ft in range(NF) if ft not in DV]
    _interleave([d_mstep(ft, j) for ft in dm for j in range(NM)], d_stream.steps())
    if DV:
        ys = [y + _rowsum(v) for y, v in zip(ys, yv)]
    for j in range(NM):
        xo = base[j] + (zero[j] + ys[j] * sig)
        o_ref[:, 128 * j:128 * (j + 1)] = xo[0:1, :].astype(o_ref.dtype)


@jax.jit
def pallas_interleave_layers__compressed_kv_cla__moe_arch_mod__decode_kernel(
        A_x, A_c_kv, A_w_q, A_w_uk, A_w_uv, A_w_o, B_x, B_w_r, B_w_gate, B_w_up, B_w_down):
    del B_x
    any_spec = pl.BlockSpec(memory_space=pl.ANY)

    def tiles(n):
        return pltpu.VMEM((max(n, 1), 64, 128), I32)

    def vregs(n):
        return pltpu.VMEM((max(n, 1), 8, 128), F32)

    out = pl.pallas_call(
        _kernel,
        out_shape=jax.ShapeDtypeStruct((1, M), BF16),
        in_specs=[any_spec] * 10,
        out_specs=pl.BlockSpec(memory_space=pltpu.VMEM),
        scratch_shapes=[
            pltpu.VMEM((1, M), BF16), pltpu.VMEM((M,), BF16),
            pltpu.VMEM((SK, DC), BF16),
            pltpu.VMEM((M * H, D), BF16), pltpu.VMEM((DC * H, D), BF16), pltpu.VMEM((DC * H, D), BF16),
            pltpu.VMEM((H * D, M), BF16),
            pltpu.VMEM((F, M), BF16), pltpu.VMEM((F, M), BF16), pltpu.VMEM((F, M), BF16),
            tiles(H * NM), tiles(H * NC),
            tiles(len(QM) * NC), vregs(len(QV) * 16 * NC),
            tiles(len(VM) * NC), vregs(len(VV) * 16 * NC),
            tiles(len(OM) * NM), vregs(len(OV) * 16 * NM),
            tiles(NC * NK),
            tiles(2 * len(GM) * NM), vregs(len(GV_TILES) * 16 * NM),
            pltpu.VMEM((NK, H, 128), F32), pltpu.VMEM((NC, H, 128), F32), pltpu.VMEM((2 * H, D), BF16),
            pltpu.VMEM((H, DC), F32), pltpu.VMEM((H, D), F32), vregs(len(VV)), pltpu.VMEM((H, D), F32),
            pltpu.VMEM((2 * NF, 8, 128), F32),
            pltpu.SemaphoreType.DMA((9 + NWO + NWD,)),
        ],
        compiler_params=pltpu.CompilerParams(vmem_limit_bytes=110 * 2**20, disable_semaphore_checks=True),
    )(A_x.reshape(1, M), B_w_r, A_c_kv.reshape(SK, DC), A_w_q.reshape(M * H, D),
      A_w_uk.reshape(DC * H, D), A_w_uv.reshape(DC * H, D), A_w_o.reshape(H * D, M),
      B_w_gate.T, B_w_up.T, B_w_down)
    return out.reshape(1, 1, M)
```
